```python
import os as _os
_os.environ.setdefault("JAX_PLATFORMS", "cpu")
import jax
import jax.numpy as jnp

def _softmax(x, axis=-1):
    return jax.nn.softmax(x, axis=axis)
def _gelu(x):
    return jax.nn.gelu(x, approximate=True)
def _silu(x):
    return jax.nn.silu(x)
def _sigmoid(x):
    return jax.nn.sigmoid(x)
def _layernorm(x, axis=-1, eps=1e-5):
    m = jnp.mean(x, axis=axis, keepdims=True)
    v = jnp.var(x, axis=axis, keepdims=True)
    return (x - m) / jnp.sqrt(v + eps)
def _scatter_add(tgt, idx, src, axis=0):
    return tgt.at[idx].add(src)
def _segment_sum(src, seg, n):
    return jax.ops.segment_sum(src, seg, n)
class _Rng:
    def __init__(self, key):
        self._k = key
    def _next(self):
        self._k, sub = jax.random.split(self._k)
        return sub
    def normal(self, shape):
        return jax.random.normal(self._next(), shape, dtype=jnp.bfloat16)
    def randint(self, lo, hi, shape):
        return jax.random.randint(self._next(), shape, lo, hi, dtype=jnp.int32)
    def uniform(self, shape, lo=0.0, hi=1.0):
        return jax.random.uniform(self._next(), shape, jnp.bfloat16, lo, hi)
    def permutation(self, n):
        return jax.random.permutation(self._next(), n)


kernel_name = 'gated_mix__mha_block__mixer_s_mlp__prompt'

def setup_inputs():
    _rng = _Rng(jax.random.key(int.from_bytes(__import__("os").urandom(4), "little")))
    _w = (lambda a: (lambda t: t.astype(jnp.bfloat16) if jnp.issubdtype(t.dtype, jnp.floating) else t)(jnp.asarray(a)))
    def _A_setup():
        B, S, D, H = 1, 2048, 448, 16
        return {
            "x": _w((lambda *s: _rng.normal(s) * 0.05)(B, S, D)),
            "wqkv": _w((lambda *s: _rng.normal(s) * 0.8)(D, 3 * D)),
            "wo": _w((lambda *s: _rng.normal(s) * 0.05)(D, D)),
        }
    _A_in = _A_setup()

    def _B_setup():
        B, S, D, F = 1, 2048, 448, 1792
        return {
            "x":  _w((lambda *s: _rng.normal(s) * 0.05)(B, S, D)),
            "w1": _w((lambda *s: _rng.normal(s) * 0.2)(D, D) * (D ** -0.5)),
            "w2": _w((lambda *s: _rng.normal(s) * 0.2)(D, D) * (D ** -0.5)),
            "w3": _w((lambda *s: _rng.normal(s) * 0.2)(D, F) * (D ** -0.5)),
            "w4": _w((lambda *s: _rng.normal(s) * 0.2)(F, D) * (F ** -0.5)),
        }
    _B_in = _B_setup()

    return {
        "A_x": _A_in["x"],
        "A_wqkv": _A_in["wqkv"],
        "A_wo": _A_in["wo"],
        "B_x": _B_in["x"],
        "B_w1": _B_in["w1"],
        "B_w2": _B_in["w2"],
        "B_w3": _B_in["w3"],
        "B_w4": _B_in["w4"],
        "gate_w": _w((lambda *s: _rng.normal(s) * 0.05)(448) * 16.0),
    }

def reference(A_x, A_wqkv, A_wo, B_x, B_w1, B_w2, B_w3, B_w4, gate_w):
    def _A_ref(x, wqkv, wo):
        B, S, D = x.shape
        H = 16
        Dh = D // H
        qkv = (lambda x, *d: x.transpose(*d))((x @ wqkv).reshape(B, S, 3, H, Dh), 2, 0, 3, 1, 4)
        q, k, v = qkv[0], qkv[1], qkv[2]
        scores = jnp.einsum("bhqd,bhkd->bhqk", q, k) * (Dh ** -0.5)
        p = _softmax(scores, axis=-1)
        o = jnp.einsum("bhqk,bhkd->bhqd", p, v)
        return (lambda x, *d: x.transpose(*d))(o, 0, 2, 1, 3).reshape(B, S, D) @ wo

    def _B_ref(x, w1, w2, w3, w4):
        B, S, D = x.shape
        h = _gelu(_layernorm(x, axis=-1) @ w1)
        c = D // 4
        g0 = jnp.pad(h[:, :, 0*c:1*c], ((0, 0), (1, 0), (0, 0)))[:, :S, :]
        g1 = jnp.pad(h[:, :, 1*c:2*c], ((0, 0), (0, 1), (0, 0)))[:, 1:, :]
        g2 = jnp.pad(h[:, :, 2*c:3*c], ((0, 0), (2, 0), (0, 0)))[:, :S, :]
        g3 = jnp.pad(h[:, :, 3*c:   ], ((0, 0), (0, 2), (0, 0)))[:, 2:, :]
        hs = jnp.concatenate([g0, g1, g2, g3], axis=-1) @ w2
        x1 = x + hs
        h2 = _gelu(_layernorm(x1, axis=-1) @ w3) @ w4
        return x1 + h2

    x = A_x
    g = _sigmoid((x * gate_w).sum(-1, keepdims=True))
    a = _A_ref(x, A_wqkv, A_wo)
    b = _B_ref(x, B_w1, B_w2, B_w3, B_w4)
    return g * a + (1 - g) * b
```

```python
import functools
import jax
import jax.numpy as jnp
import jax.experimental.pallas as pl
import jax.experimental.pallas.tpu as pltpu

S, D, H, DH, F = 2048, 448, 16, 28, 1792
HP = 32
DP = H * HP
G = 112
TQ = 256
HS = 2
NS = H // HS
W = TQ * HS
TK = 128
NC = S // TK
CH = 512
LAG = 1
LOG2E = 1.4426950408889634
f32, bf16 = jnp.float32, jnp.bfloat16
P0 = 512


def _gelu(x):
    return jax.nn.gelu(x, approximate=True)


def _ln0(x):
    m = jnp.mean(x, axis=0, keepdims=True)
    xc = x - m
    v = jnp.mean(xc * xc, axis=0, keepdims=True)
    return xc * jax.lax.rsqrt(v + 1e-5)


def _dot(a, b):
    return jnp.dot(a, b, preferred_element_type=f32)


def kernel(xt_hbm, wqkv_hbm, wo_hbm, w1_hbm, w2_hbm, w3_hbm, w4t_hbm, gw_ref,
           o_ref,
           xt_ref, wqkv_ref, wo_ref, w1_ref, w2_ref, w3_ref, w4t_ref, sems,
           wqkvt_sc, w1t_sc, w2t_sc, w3t_sc, wot_sc, gwc_sc,
           q_sc, k_sc, vt_sc, h_sc, hs_sc, ot_sc, h3_sc, sa, sb):
    i = pl.program_id(0)

    @pl.when(i == 0)
    def _():
        def cp(src, dst, n):
            return pltpu.make_async_copy(src, dst, sems.at[n])
        cw0 = cp(wqkv_hbm.at[:, 0:P0], wqkv_ref.at[:, 0:P0], 0)
        cw1 = cp(wqkv_hbm.at[:, P0:], wqkv_ref.at[:, P0:], 1)
        cx0 = cp(xt_hbm.at[:, 0:CH], xt_ref.at[:, 0:CH], 2)
        cx1 = cp(xt_hbm.at[:, CH:], xt_ref.at[:, CH:], 3)
        c1, c2, c3, c4, co = (cp(w1_hbm, w1_ref, 4), cp(w2_hbm, w2_ref, 5), cp(w3_hbm, w3_ref, 6),
                              cp(w4t_hbm, w4t_ref, 7), cp(wo_hbm, wo_ref, 8))
        for c in (cw0, cx0, cw1, c1, cx1, c2, co, c3, c4):
            c.start()
        sa[0:8, :] = jnp.zeros((8, W), f32)
        sb[0:8, :] = jnp.zeros((8, W), f32)
        gwc_sc[...] = jnp.broadcast_to(gw_ref[...].astype(f32), (128, D)).T

        z16 = jnp.zeros((128 - G, CH), bf16)
        tail = jnp.where(jax.lax.broadcasted_iota(jnp.int32, (HP - DH, CH), 0) == 0, 1.0, 0.0).astype(f32)

        def do_q(cs):
            q_sc[:, cs] = (_dot(wqkvt_sc[0:D, :], xt_ref[:, cs]) * (DH ** -0.5 * LOG2E)).astype(bf16)

        def do_kv(cs):
            kv = _dot(wqkvt_sc[D:, :], xt_ref[:, cs])
            for g in range(4):
                kg = jnp.concatenate([kv[g * G:(g + 1) * G].astype(bf16), z16], axis=0)
                k_sc[g, cs, :] = kg.T
            for h in range(H):
                vh = jnp.concatenate([kv[D + h * DH:D + (h + 1) * DH], tail], axis=0)
                vt_sc[h, :, cs] = vh.astype(bf16)

        def do_h(cs):
            xn = _ln0(xt_ref[:, cs].astype(f32)).astype(bf16)
            h_sc[:, cs] = _gelu(_dot(w1t_sc[...], xn))

        chunk = lambda c: slice(c * CH, (c + 1) * CH)
        cw0.wait()
        cx0.wait()
        wqkvt_sc[0:P0, :] = wqkv_ref[:, 0:P0].T
        do_q(chunk(0))
        cw1.wait()
        c1.wait()
        wqkvt_sc[P0:, :] = wqkv_ref[:, P0:].T
        w1t_sc[...] = w1_ref[...].T
        do_kv(chunk(0))
        do_h(chunk(0))
        cx1.wait()
        c2.wait()
        co.wait()
        do_q(chunk(1))
        w2t_sc[...] = w2_ref[...].T
        wo = wo_ref[...].astype(f32)
        z4 = jnp.zeros((HP - DH, D), f32)
        wop = jnp.concatenate([p for h in range(H) for p in (wo[h * DH:(h + 1) * DH], z4)], axis=0)
        wot_sc[...] = wop.astype(bf16).T
        do_h(chunk(1))
        do_kv(chunk(1))
        c3.wait()
        c4.wait()
        do_q(chunk(2))
        w3t_sc[...] = w3_ref[...].T
        do_h(chunk(2))
        do_h(chunk(3))
        do_kv(chunk(2))
        lane = jax.lax.broadcasted_iota(jnp.int32, (G, S), 1)
        for g, sh in enumerate((1, -1, 2, -2)):
            hg = h_sc[g * G:(g + 1) * G, :]
            r = pltpu.roll(hg, sh % S, axis=1)
            valid = (lane >= sh) if sh > 0 else (lane < S + sh)
            hs_sc[g * G:(g + 1) * G, :] = jnp.where(valid, r, 0.0).astype(bf16)
        do_kv(chunk(3))
        do_q(chunk(3))

    q0 = pl.multiple_of(i * TQ, TQ)
    bufs = (sa, sb)

    def masked_q(h):
        g, j = h // 4, h % 4
        lo, hi = (j * DH) // 16 * 16, -(-((j + 1) * DH) // 16) * 16
        qw = q_sc[g * G + lo:g * G + hi, pl.ds(q0, TQ)]
        row = jax.lax.broadcasted_iota(jnp.int32, (hi - lo, TQ), 0) + lo
        qw = jnp.where((row >= j * DH) & (row < (j + 1) * DH), qw, jnp.zeros_like(qw))
        parts = []
        if lo > 0:
            parts.append(jnp.zeros((lo, TQ), bf16))
        parts.append(qw)
        parts.append(jnp.zeros((128 - hi, TQ), bf16))
        return jnp.concatenate(parts, axis=0)

    def qk_chunk(st, c, qm, mpart):
        s = _dot(k_sc[st * HS // 4, c * TK:(c + 1) * TK, :], qm)
        bufs[st % 2][c * TK:(c + 1) * TK, :] = s
        sm = jnp.max(s.reshape(TK // 8, 8, W), axis=0)
        return sm if mpart is None else jnp.maximum(mpart, sm)

    def pv_chunk(st, c, m, acc):
        p = jnp.exp2(bufs[st % 2][c * TK:(c + 1) * TK, :] - m).astype(bf16)
        o = [_dot(vt_sc[st * HS + k, :, c * TK:(c + 1) * TK], p[:, k * TQ:(k + 1) * TQ]) for k in range(HS)]
        return o if acc is None else [x + y for x, y in zip(acc, o)]

    xf = xt_ref[:, pl.ds(q0, TQ)].astype(f32)
    x1 = xf + _dot(w2t_sc[...], hs_sc[:, pl.ds(q0, TQ)])
    x1n = _ln0(x1).astype(bf16)
    gl = jnp.sum(xf * jnp.tile(gwc_sc[...], (1, TQ // 128)), axis=0, keepdims=True)
    g = jax.nn.sigmoid(gl)

    FC = F // NC
    off = NC + LAG
    ms, mpart, accs, qms = {}, {}, {}, {}
    for t in range(NS * NC + off):
        if t < NS * NC:
            st, c = divmod(t, NC)
            if c == 0:
                qms[st] = jnp.concatenate([masked_q(st * HS + k) for k in range(HS)], axis=1)
            mpart[st] = qk_chunk(st, c, qms[st], mpart.get(st))
            if c == NC - 1:
                ms[st] = jnp.max(mpart[st], axis=0, keepdims=True)
        elif t - NS * NC < NC:
            c = t - NS * NC
            h3_sc[c * FC:(c + 1) * FC, :] = _gelu(_dot(w3t_sc[c * FC:(c + 1) * FC, :], x1n)).astype(bf16)
        u = t - off
        if u >= 0:
            st, c = divmod(u, NC)
            accs[st] = pv_chunk(st, c, ms[st], accs.get(st))
            if c == NC - 1:
                for k in range(HS):
                    acc = accs[st][k]
                    ot_sc[st * HS + k] = (acc * (1.0 / acc[DH:DH + 1, :])).astype(bf16)

    b = x1 + _dot(w4t_ref[...], h3_sc[...])
    a = _dot(wot_sc[...], ot_sc[...].reshape(DP, TQ))
    o_ref[...] = (g * a + (1.0 - g) * b).astype(o_ref.dtype)


@jax.jit
def pallas_gated_mix__mha_block__mixer_s_mlp__prompt_kernel(A_x, A_wqkv, A_wo, B_x, B_w1, B_w2, B_w3, B_w4, gate_w):
    xt = A_x.reshape(S, D).T
    gw = gate_w.reshape(1, D)
    anyspec = pl.BlockSpec(memory_space=pl.ANY)
    ins = (xt, A_wqkv, A_wo, B_w1, B_w2, B_w3, B_w4.T, gw)
    out = pl.pallas_call(
        kernel,
        grid=(S // TQ,),
        in_specs=[anyspec] * 7 + [pl.BlockSpec((1, D), lambda i: (0, 0))],
        out_specs=pl.BlockSpec((D, TQ), lambda i: (0, i)),
        out_shape=jax.ShapeDtypeStruct((D, S), bf16),
        scratch_shapes=[
            pltpu.VMEM((D, S), bf16), pltpu.VMEM((D, 3 * D), bf16), pltpu.VMEM((D, D), bf16),
            pltpu.VMEM((D, D), bf16), pltpu.VMEM((D, D), bf16), pltpu.VMEM((D, F), bf16), pltpu.VMEM((D, F), bf16),
            pltpu.SemaphoreType.DMA((9,)),
            pltpu.VMEM((3 * D, D), bf16), pltpu.VMEM((D, D), bf16), pltpu.VMEM((D, D), bf16),
            pltpu.VMEM((F, D), bf16), pltpu.VMEM((D, DP), bf16), pltpu.VMEM((D, 128), f32),
            pltpu.VMEM((D, S), bf16), pltpu.VMEM((4, S, 128), bf16), pltpu.VMEM((H, HP, S), bf16),
            pltpu.VMEM((D, S), f32), pltpu.VMEM((D, S), bf16), pltpu.VMEM((H, HP, TQ), bf16),
            pltpu.VMEM((F, TQ), bf16),
            pltpu.VMEM((S, W), f32), pltpu.VMEM((S, W), f32),
        ],
        compiler_params=pltpu.CompilerParams(dimension_semantics=("arbitrary",), vmem_limit_bytes=100 * 1024 * 1024),
        name="gm",
    )(*ins)
    return out.T.reshape(1, S, D)
```

```python
import functools

import jax
import jax.numpy as jnp
import jax.experimental.pallas as pl
import jax.experimental.pallas.tpu as pltpu

S, D, H, DH, F = 2048, 448, 16, 28, 1792
HP = 32
DP = H * HP
G = 112
TQ = 256
HS = 2
NS = H // HS
W = TQ * HS
TK = 128
NC = S // TK
CH = 512
LAG = 1
X1_AT, W3_AT, W4_STEP = 1, 10, 4
PORDER = (1, 3, 2, 4, 0, 6, 5)
P0 = 512
D2, F2, T2, C2 = D // 2, F // 2, TQ // 2, CH // 2
LOG2E = 1.4426950408889634
EPS = 1e-5
f32, bf16 = jnp.float32, jnp.bfloat16


def _gelu2(x):
    c = 0.7978845608028654
    return x + x * jnp.tanh(x * (c + (c * 0.044715) * (x * x)))


def _ln_stats(x):
    m = jnp.mean(x, axis=0, keepdims=True)
    var = jnp.maximum(jnp.mean(x * x, axis=0, keepdims=True) - m * m, 0.0)
    return m, jax.lax.rsqrt(var + EPS)


def _dot(a, b):
    return jnp.dot(a, b, preferred_element_type=f32)


_LHS = (((0, 0), (1, 1), 1), ((1, 0), (1, 1), 1), ((0, 0), None, 0), ((1, 1), None, 0),
        ((0, 0), (0, 1), 1), ((1, 0), (0, 0), -1), ((0, 1), (1, 1), -1))
_RHS = (((0, 0), (1, 1), 1), ((0, 0), None, 0), ((0, 1), (1, 1), -1), ((1, 0), (0, 0), -1),
        ((1, 1), None, 0), ((0, 0), (0, 1), 1), ((1, 0), (1, 1), 1))


def _st_operand(table, blk, n):
    p, q, sign = table[n]
    if q is None:
        return blk(*p).astype(bf16)
    u, v = blk(*p).astype(f32), blk(*q).astype(f32)
    return (u + v if sign > 0 else u - v).astype(bf16)


_st_lhs = functools.partial(_st_operand, _LHS)
_st_rhs = functools.partial(_st_operand, _RHS)


def _st_out(m):
    return (m[0] + m[3] - m[4] + m[6], m[2] + m[4], m[1] + m[3], m[0] - m[1] + m[2] + m[5])


def _st_join(c):
    return jnp.concatenate([jnp.concatenate(c[:2], axis=1), jnp.concatenate(c[2:], axis=1)], axis=0)


def _kernel(xt_hbm, wqkv_hbm, wo_hbm, w1_hbm, w2_hbm, w3_hbm, w4t_hbm, gw_hbm,
            o_ref,
            xt_ref, wqkv_ref, wo_ref, w1_ref, w2_ref, w3_ref, w4t_ref, gw_ref, sems,
            wt_s, w1_o, w1_s, w2_s, w3_s, wo_s, gwc_sc,
            q_sc, k_sc, vt_sc, h_sc, hs_sc, ot_sc, h3_sc, x1_sc, fz_sc, sa, sb):
    i = pl.program_id(0)
    half_blk = lambda r: (lambda a, b: r[b, a * D2:(a + 1) * D2, :])

    def fence():
        fz_sc[...] = jnp.zeros((8, 128), f32)

    def products(lhs, rhs):
        m = [None] * 7
        for n in PORDER:
            m[n] = _dot(lhs(n), rhs(n))
            fence()
        return m

    @pl.when(i == 0)
    def _():
        def cp(src, dst, n):
            return pltpu.make_async_copy(src, dst, sems.at[n])
        cw0 = cp(wqkv_hbm.at[:, 0:P0], wqkv_ref.at[:, 0:P0], 0)
        cw1 = cp(wqkv_hbm.at[:, P0:], wqkv_ref.at[:, P0:], 1)
        cx0 = cp(xt_hbm.at[:, 0:CH], xt_ref.at[:, 0:CH], 2)
        cx1 = cp(xt_hbm.at[:, CH:], xt_ref.at[:, CH:], 3)
        c1, c2, c3, c4, co, cg = (cp(w1_hbm, w1_ref, 4), cp(w2_hbm, w2_ref, 5), cp(w3_hbm, w3_ref, 6),
                                  cp(w4t_hbm, w4t_ref, 7), cp(wo_hbm, wo_ref, 8), cp(gw_hbm, gw_ref, 9))
        for c in (cg, cw0, cx0, cw1, cx1, c1, c3, c2, co, c4):
            c.start()
        sa[0:8, :] = jnp.zeros((8, W), f32)
        x1_sc[0:8, :] = jnp.zeros((8, TQ), f32)
        sb[0:8, :] = jnp.zeros((8, W), f32)
        cg.wait()
        gwc_sc[...] = jnp.broadcast_to(gw_ref[...].astype(f32).reshape(1, D), (128, D)).T

        z16 = jnp.zeros((128 - G, CH), bf16)
        tail = jnp.where(jax.lax.broadcasted_iota(jnp.int32, (HP - DH, CH), 0) == 0, 1.0, 0.0).astype(f32)
        chunk = lambda c: slice(c * CH, (c + 1) * CH)
        never = jax.lax.broadcasted_iota(jnp.int32, (D, CH), 1) < i
        stats = {}

        def proj(w, c, fast):
            if not fast:
                return (_dot(wt_s[0, w * D:(w + 1) * D, :], xt_ref[0:D2, chunk(c)])
                        + _dot(wt_s[1, w * D:(w + 1) * D, :], xt_ref[D2:, chunk(c)]))
            ablk = lambda a, b: wt_s[b, w * D + a * D2:w * D + (a + 1) * D2, :]
            xblk = lambda a, b: xt_ref[a * D2:(a + 1) * D2, c * CH + b * C2:c * CH + (b + 1) * C2]
            return _st_join(_st_out(products(lambda n: _st_lhs(ablk, n), lambda n: _st_rhs(xblk, n))))

        def do_q(c):
            q_sc[:, chunk(c)] = (proj(0, c, False) * (DH ** -0.5 * LOG2E)).astype(bf16)

        def do_k(c):
            cs = chunk(c)
            kt = proj(1, c, False)
            stats[c] = _ln_stats(jnp.where(never, kt, xt_ref[:, cs].astype(f32)))
            for g in range(4):
                kg = jnp.concatenate([kt[g * G:(g + 1) * G].astype(bf16), z16], axis=0)
                k_sc[g, cs, :] = kg.T

        def do_v(c):
            vt = proj(2, c, c > 0)
            for h in range(H):
                vh = jnp.concatenate([vt[h * DH:(h + 1) * DH], tail], axis=0)
                vt_sc[h, :, chunk(c)] = vh.astype(bf16)

        def do_h(c):
            m, r = stats[c]
            nblk = lambda a, b: ((xt_ref[a * D2:(a + 1) * D2, c * CH + b * C2:c * CH + (b + 1) * C2].astype(f32)
                                  - m[:, b * C2:(b + 1) * C2]) * r[:, b * C2:(b + 1) * C2])
            y = products(lambda n: w1_o[n], lambda n: _st_rhs(nblk, n))
            h_sc[:, chunk(c)] = _gelu2(_st_join(_st_out(y)))

        def prep_w3(j):
            blk = lambda a, b: w3_ref[b * D2:(b + 1) * D2, a * F2 + j * 128:a * F2 + (j + 1) * 128]
            for n in range(7):
                w3_s[n, j * 128:(j + 1) * 128, :] = _st_lhs(blk, n).T

        def halves_t(w, dst):
            k2 = w.shape[0] // 2
            dst[0] = w[:k2].T
            dst[1] = w[k2:].T

        def prep_wo():
            wo = wo_ref[...].astype(f32)
            z4 = jnp.zeros((HP - DH, D), f32)
            wop = jnp.concatenate([p for h in range(H) for p in (wo[h * DH:(h + 1) * DH], z4)], axis=0)
            halves_t(wop.astype(bf16), wo_s)

        def shift(g):
            sh = (1, -1, 2, -2)[g]
            lane = jax.lax.broadcasted_iota(jnp.int32, (G, S), 1)
            r = pltpu.roll(h_sc[g * G:(g + 1) * G, :], sh % S, axis=1)
            valid = (lane >= sh) if sh > 0 else (lane < S + sh)
            hs_sc[g * G:(g + 1) * G, :] = jnp.where(valid, r, 0.0)

        cw0.wait()
        for b in range(2):
            wt_s[b, 0:P0, :] = wqkv_ref[b * D2:(b + 1) * D2, 0:P0].T
        cx0.wait()
        do_q(0)
        cw1.wait()
        for b in range(2):
            wt_s[b, P0:, :] = wqkv_ref[b * D2:(b + 1) * D2, P0:].T
        do_k(0)
        do_v(0)
        cx1.wait()
        c1.wait()
        halves_t(w1_ref[...], w1_s)
        for n in range(7):
            w1_o[n] = _st_lhs(half_blk(w1_s), n)
        for f, c in ((do_k, 1), (do_k, 2), (do_h, 0), (do_v, 1), (do_k, 3), (do_h, 1), (do_v, 2)):
            f(c)
        c3.wait()
        c2.wait()
        co.wait()
        c4.wait()
        do_q(1)
        do_q(2)
        for j in range(F2 // 128):
            prep_w3(j)
        halves_t(w2_ref[...], w2_s)
        prep_wo()
        do_h(2)
        do_v(3)
        do_h(3)
        for g in range(4):
            shift(g)
        do_q(3)

    q0 = pl.multiple_of(i * TQ, TQ)
    bufs = (sa, sb)

    def masked_q(h):
        g, j = h // 4, h % 4
        lo, hi = (j * DH) // 16 * 16, -(-((j + 1) * DH) // 16) * 16
        qw = q_sc[g * G + lo:g * G + hi, pl.ds(q0, TQ)]
        row = jax.lax.broadcasted_iota(jnp.int32, (hi - lo, TQ), 0) + lo
        qw = jnp.where((row >= j * DH) & (row < (j + 1) * DH), qw, jnp.zeros_like(qw))
        parts = []
        if lo > 0:
            parts.append(jnp.zeros((lo, TQ), bf16))
        parts.append(qw)
        parts.append(jnp.zeros((128 - hi, TQ), bf16))
        return jnp.concatenate(parts, axis=0)

    def qk_chunk(st, c, qm, mpart):
        s = _dot(k_sc[st * HS // 4, c * TK:(c + 1) * TK, :], qm)
        bufs[st % 2][c * TK:(c + 1) * TK, :] = s
        sm = jnp.max(s.reshape(TK // 8, 8, W), axis=0)
        return sm if mpart is None else jnp.maximum(mpart, sm)

    def pv_chunk(st, c, m, acc):
        o = []
        for k in range(HS):
            sl = slice(k * TQ, (k + 1) * TQ)
            p = jnp.exp2(bufs[st % 2][c * TK:(c + 1) * TK, sl] - m[:, sl]).astype(bf16)
            o.append(_dot(vt_sc[st * HS + k, :, c * TK:(c + 1) * TK], p))
        return o if acc is None else [x + y for x, y in zip(acc, o)]

    env = {}

    def do_x1():
        hblk = lambda a, b: hs_sc[a * D2:(a + 1) * D2, pl.ds(pl.multiple_of(q0 + b * T2, T2), T2)]
        m2 = products(lambda n: _st_lhs(half_blk(w2_s), n), lambda n: _st_rhs(hblk, n))
        xf = xt_ref[:, pl.ds(q0, TQ)].astype(f32)
        x1 = xf + 0.5 * _st_join(_st_out(m2))
        x1_sc[...] = x1
        env['m'], env['r'] = _ln_stats(x1)
        gl = jnp.sum(xf * jnp.tile(gwc_sc[...], (1, TQ // 128)), axis=0, keepdims=True)
        env['g'] = jax.nn.sigmoid(gl)

    def do_w3():
        nblk = lambda a, b: ((x1_sc[a * D2:(a + 1) * D2, b * T2:(b + 1) * T2] - env['m'][:, b * T2:(b + 1) * T2])
                             * env['r'][:, b * T2:(b + 1) * T2])
        m3 = products(lambda n: w3_s[n], lambda n: _st_rhs(nblk, n))
        h3 = [_gelu2(v) for v in _st_out(m3)]
        for n in range(7):
            h3_sc[n] = _st_rhs(lambda a, b: h3[2 * a + b], n)

    m4 = [None] * 7

    def do_w4(n):
        blk = lambda a, b: w4t_ref[a * D2:(a + 1) * D2, b * F2:(b + 1) * F2]
        m4[n] = _dot(_st_lhs(blk, n), h3_sc[n])
        fence()

    t_qk = NS * NC
    off = NC + LAG
    extra = {X1_AT: [do_x1], W3_AT: [do_w3]}
    for n in range(7):
        slot = min(t_qk - 1 + n * W4_STEP, t_qk + off - 1)
        extra.setdefault(slot, []).append(functools.partial(do_w4, PORDER[n]))

    ms, mpart, accs, qms = {}, {}, {}, {}
    for t in range(t_qk + off):
        if t < t_qk:
            st, c = divmod(t, NC)
            if c == 0:
                qms[st] = jnp.concatenate([masked_q(st * HS + k) for k in range(HS)], axis=1)
            mpart[st] = qk_chunk(st, c, qms[st], mpart.get(st))
            if c == NC - 1:
                ms[st] = jnp.max(mpart[st], axis=0, keepdims=True)
        u = t - off
        if u >= 0:
            st, c = divmod(u, NC)
            accs[st] = pv_chunk(st, c, ms[st], accs.get(st))
            if c == NC - 1:
                for k in range(HS):
                    acc = accs[st][k]
                    ot_sc[st * HS + k] = acc * (1.0 / acc[DH:DH + 1, :])
        for f in extra.get(t, ()):
            f()

    oblk = lambda a, b: ot_sc[a * (H // 2):(a + 1) * (H // 2), :, b * T2:(b + 1) * T2].reshape(DP // 2, T2)
    mo = products(lambda n: _st_lhs(half_blk(wo_s), n), lambda n: _st_rhs(oblk, n))
    b = x1_sc[...] + 0.5 * _st_join(_st_out(m4))
    a = _st_join(_st_out(mo))
    g = env['g']
    o_ref[...] = (g * a + (1.0 - g) * b).astype(o_ref.dtype)


@jax.jit
def pallas_gated_mix__mha_block__mixer_s_mlp__prompt_kernel(
    A_x: jax.Array,
    A_wqkv: jax.Array,
    A_wo: jax.Array,
    B_x: jax.Array,
    B_w1: jax.Array,
    B_w2: jax.Array,
    B_w3: jax.Array,
    B_w4: jax.Array,
    gate_w: jax.Array,
):
    del B_x
    xt = A_x.reshape(S, D).T
    vm = pltpu.VMEM
    out = pl.pallas_call(
        _kernel,
        grid=(S // TQ,),
        in_specs=[pl.BlockSpec(memory_space=pl.ANY)] * 8,
        out_specs=pl.BlockSpec((D, TQ), lambda i: (0, i)),
        out_shape=jax.ShapeDtypeStruct((D, S), bf16),
        scratch_shapes=[
            vm((D, S), bf16), vm((D, 3 * D), bf16), vm((D, D), bf16), vm((D, D), bf16), vm((D, D), bf16),
            vm((D, F), bf16), vm((D, F), bf16), vm((D,), bf16), pltpu.SemaphoreType.DMA((10,)),
            vm((2, 3 * D, D2), bf16), vm((7, D2, D2), bf16), vm((2, D, D2), bf16), vm((2, D, D2), bf16),
            vm((7, F2, D2), bf16), vm((2, D, DP // 2), bf16), vm((D, 128), f32),
            vm((D, S), bf16), vm((4, S, 128), bf16), vm((H, HP, S), bf16),
            vm((D, S), f32), vm((D, S), f32), vm((H, HP, TQ), f32),
            vm((7, F2, T2), bf16), vm((D, TQ), f32), vm((8, 128), f32),
            vm((S, W), f32), vm((S, W), f32),
        ],
        compiler_params=pltpu.CompilerParams(dimension_semantics=("arbitrary",),
                                             vmem_limit_bytes=100 * 1024 * 1024),
        name="gm",
    )(xt, A_wqkv, A_wo, B_w1, B_w2, B_w3, B_w4.T, gate_w)
    return out.T.reshape(1, S, D)
```

```python
import functools

import jax
import jax.numpy as jnp
import jax.experimental.pallas as pl
import jax.experimental.pallas.tpu as pltpu

S, D, H, DH, F = 2048, 448, 16, 28, 1792
HP = 32
DP = H * HP
G = 112
TQ = 256
HS = 2
NS = H // HS
W = TQ * HS
TK = 128
NC = S // TK
CH = 512
LAG = 1
X1_AT, W3_AT, W4_STEP = 1, 12, 4
PORDER = (1, 3, 2, 4, 0, 6, 5)
P0 = 512
D2, F2, T2, C2 = D // 2, F // 2, TQ // 2, CH // 2
LOG2E = 1.4426950408889634
EPS = 1e-5
f32, bf16 = jnp.float32, jnp.bfloat16


def _gelu2(x):
    c = 0.7978845608028654
    return x + x * jnp.tanh(x * (c + (c * 0.044715) * (x * x)))


def _ln_stats(x):
    m = jnp.mean(x, axis=0, keepdims=True)
    var = jnp.maximum(jnp.mean(x * x, axis=0, keepdims=True) - m * m, 0.0)
    return m, jax.lax.rsqrt(var + EPS)


def _dot(a, b):
    return jnp.dot(a, b, preferred_element_type=f32)


_LHS = (((0, 0), (1, 1), 1), ((1, 0), (1, 1), 1), ((0, 0), None, 0), ((1, 1), None, 0),
        ((0, 0), (0, 1), 1), ((1, 0), (0, 0), -1), ((0, 1), (1, 1), -1))
_RHS = (((0, 0), (1, 1), 1), ((0, 0), None, 0), ((0, 1), (1, 1), -1), ((1, 0), (0, 0), -1),
        ((1, 1), None, 0), ((0, 0), (0, 1), 1), ((1, 0), (1, 1), 1))


def _st_operand(table, blk, n):
    p, q, sign = table[n]
    if q is None:
        return blk(*p).astype(bf16)
    u, v = blk(*p).astype(f32), blk(*q).astype(f32)
    return (u + v if sign > 0 else u - v).astype(bf16)


_st_lhs = functools.partial(_st_operand, _LHS)
_st_rhs = functools.partial(_st_operand, _RHS)


def _st_out(m):
    return (m[0] + m[3] - m[4] + m[6], m[2] + m[4], m[1] + m[3], m[0] - m[1] + m[2] + m[5])


def _st_join(c):
    return jnp.concatenate([jnp.concatenate(c[:2], axis=1), jnp.concatenate(c[2:], axis=1)], axis=0)


_HT = (0.0, 1.0, -1.0, 2.0)
_HK = []
for _j in range(4):
    _new = [('P', _j, _j), ('Q', _j, _j)]
    for _i in range(_j + 1, 4):
        _new = [('M', _j, _i), ('T', _j, _i), ('T', _i, _j)] + _new
    _HK += _new


def _lin(terms):
    acc = None
    for c, v in sorted([t for t in terms if t[0] != 0.0], key=lambda t: t[0] < 0):
        x = v()
        if abs(c) != 1.0:
            x = x * abs(c)
        if acc is None:
            acc = x if c > 0 else -x
        else:
            acc = acc + x if c > 0 else acc - x
    return acc


def _hk_lhs(blk, p):
    kind, i, j = p
    f = lambda a, b: (lambda: blk(a, b).astype(f32))
    if kind == 'T':
        return blk(j, i).astype(bf16)
    if kind == 'M':
        return _lin([(1.0, f(j, i)), (1.0, f(i, j))]).astype(bf16)
    if kind == 'P':
        return _lin([(1.0 if r == i else -1.0, f(r, i)) for r in range(4)]).astype(bf16)
    return _lin([(1.0, f(i, r)) for r in range(4)]).astype(bf16)


def _hk_rhs_coef(p):
    kind, i, j = p
    if kind == 'P':
        return {i: 1.0}, {}, 1.0
    if kind == 'Q':
        return {i: _HT[i]}, {i: 1.0}, 1.0
    d = _HT[i] - _HT[j]
    sg = 1.0 if d > 0 else -1.0
    if kind == 'M':
        return {i: sg * _HT[i], j: -sg * _HT[j]}, {i: sg, j: -sg}, abs(d)
    return {j: sg * _HT[j], i: -sg * _HT[j]}, {j: sg, i: -sg}, abs(d)


def _hk_rhs_ln(blk, m, r, p):
    c0, c1, d = _hk_rhs_coef(p)
    acc, off = None, None
    for n, c in enumerate((c0, c1)):
        c = {k: v for k, v in c.items() if v != 0.0}
        if not c:
            continue
        g = min(abs(v) for v in c.values())
        if all(v < 0 for v in c.values()):
            g = -g
        rs = r[n] * (g / d)
        x = _lin([(v / g, functools.partial(blk, k, n)) for k, v in c.items()]) * rs
        acc = x if acc is None else acc + x
        tot = sum(c.values()) / g
        if tot != 0.0:
            o = m[n] * rs * tot
            off = o if off is None else off + o
    return (acc if off is None else acc - off).astype(bf16)


def _hk_out(m, j):
    k = lambda v: (lambda: v)
    others = [i for i in range(4) if i != j]
    gjj = _lin([(1.0, k(m['M', min(i, j), max(i, j)])) for i in others] + [(1.0, k(m['T', j, i])) for i in others]
               + [(1.0, k(m['P', j, j]))])
    z0 = _lin([(1.0, k(m['T', i, j])) for i in others] + [(1.0, k(gjj))])
    z1 = _lin([(1.0, k(m['Q', j, j]))] + [(-_HT[i], k(m['T', i, j])) for i in others] + [(-_HT[j], k(gjj))])
    return z0, z1


def _kernel(xt_hbm, wqkv_hbm, wo_hbm, w1_hbm, w2_hbm, w3_hbm, w4t_hbm, gw_hbm,
            o_ref,
            xt_ref, wqkv_ref, wo_ref, w1_ref, w2_ref, w3_ref, w4t_ref, gw_ref, sems,
            wt_s, w1_o, w1_s, w2_s, w3_s, wo_s, gwc_sc,
            q_sc, k_sc, vt_sc, h_sc, hs_sc, ot_sc, h3_sc, hf_sc, x1_sc, fz_sc, sa, sb):
    i = pl.program_id(0)
    half_blk = lambda r: (lambda a, b: r[b, a * D2:(a + 1) * D2, :])

    def fence():
        fz_sc[...] = jnp.zeros((8, 128), f32)

    def products(lhs, rhs):
        m = [None] * 7
        for n in PORDER:
            m[n] = _dot(lhs(n), rhs(n))
            fence()
        return m

    @pl.when(i == 0)
    def _():
        def cp(src, dst, n):
            return pltpu.make_async_copy(src, dst, sems.at[n])
        cw0 = cp(wqkv_hbm.at[:, 0:P0], wqkv_ref.at[:, 0:P0], 0)
        cw1 = cp(wqkv_hbm.at[:, P0:], wqkv_ref.at[:, P0:], 1)
        cx0 = cp(xt_hbm.at[:, 0:CH], xt_ref.at[:, 0:CH], 2)
        cx1 = cp(xt_hbm.at[:, CH:], xt_ref.at[:, CH:], 3)
        c1, c2, c3, c4, co, cg = (cp(w1_hbm, w1_ref, 4), cp(w2_hbm, w2_ref, 5), cp(w3_hbm, w3_ref, 6),
                                  cp(w4t_hbm, w4t_ref, 7), cp(wo_hbm, wo_ref, 8), cp(gw_hbm, gw_ref, 9))
        for c in (cg, cw0, cx0, cw1, cx1, c1, c3, c2, co, c4):
            c.start()
        sa[0:8, :] = jnp.zeros((8, W), f32)
        x1_sc[0:8, :] = jnp.zeros((8, TQ), f32)
        hf_sc[0, 0, 0:8, :] = jnp.zeros((8, T2), f32)
        sb[0:8, :] = jnp.zeros((8, W), f32)
        cg.wait()
        gwc_sc[...] = jnp.broadcast_to(gw_ref[...].astype(f32).reshape(1, D), (128, D)).T

        z16 = jnp.zeros((128 - G, CH), bf16)
        tail = jnp.where(jax.lax.broadcasted_iota(jnp.int32, (HP - DH, CH), 0) == 0, 1.0, 0.0).astype(f32)
        chunk = lambda c: slice(c * CH, (c + 1) * CH)
        never = jax.lax.broadcasted_iota(jnp.int32, (D, CH), 1) < i
        stats = {}

        def proj(w, c, fast):
            if not fast:
                return (_dot(wt_s[0, w * D:(w + 1) * D, :], xt_ref[0:D2, chunk(c)])
                        + _dot(wt_s[1, w * D:(w + 1) * D, :], xt_ref[D2:, chunk(c)]))
            ablk = lambda a, b: wt_s[b, w * D + a * D2:w * D + (a + 1) * D2, :]
            xblk = lambda a, b: xt_ref[a * D2:(a + 1) * D2, c * CH + b * C2:c * CH + (b + 1) * C2]
            return _st_join(_st_out(products(lambda n: _st_lhs(ablk, n), lambda n: _st_rhs(xblk, n))))

        def do_q(c):
            q_sc[:, chunk(c)] = (proj(0, c, False) * (DH ** -0.5 * LOG2E)).astype(bf16)

        def do_k(c):
            cs = chunk(c)
            kt = proj(1, c, False)
            stats[c] = _ln_stats(jnp.where(never, kt, xt_ref[:, cs].astype(f32)))
            for g in range(4):
                kg = jnp.concatenate([kt[g * G:(g + 1) * G].astype(bf16), z16], axis=0)
                k_sc[g, cs, :] = kg.T

        def do_v(c):
            vt = proj(2, c, True)
            for h in range(H):
                vh = jnp.concatenate([vt[h * DH:(h + 1) * DH], tail], axis=0)
                vt_sc[h, :, chunk(c)] = vh.astype(bf16)

        def do_h(c):
            m, r = stats[c]
            nblk = lambda a, b: ((xt_ref[a * D2:(a + 1) * D2, c * CH + b * C2:c * CH + (b + 1) * C2].astype(f32)
                                  - m[:, b * C2:(b + 1) * C2]) * r[:, b * C2:(b + 1) * C2])
            y = products(lambda n: w1_o[n], lambda n: _st_rhs(nblk, n))
            h_sc[:, chunk(c)] = _gelu2(_st_join(_st_out(y)))

        def prep_w3(j):
            if j < 3:
                blk = lambda r, k: w3_ref[k * G:(k + 1) * G, r * 384 + j * 128:r * 384 + (j + 1) * 128]
                rows = slice(j * 128, (j + 1) * 128)
            else:
                blk = lambda r, k: w3_ref[k * G:(k + 1) * G, 1536 + r * 64:1536 + (r + 1) * 64]
                rows = slice(384, D)
            for n, p in enumerate(_HK):
                w3_s[n, rows, :] = _hk_lhs(blk, p).T

        def halves_t(w, dst):
            k2 = w.shape[0] // 2
            dst[0] = w[:k2].T
            dst[1] = w[k2:].T

        def prep_wo():
            wo = wo_ref[...].astype(f32)
            z4 = jnp.zeros((HP - DH, D), f32)
            wop = jnp.concatenate([p for h in range(H) for p in (wo[h * DH:(h + 1) * DH], z4)], axis=0)
            halves_t(wop.astype(bf16), wo_s)

        def shift(g):
            sh = (1, -1, 2, -2)[g]
            lane = jax.lax.broadcasted_iota(jnp.int32, (G, S), 1)
            r = pltpu.roll(h_sc[g * G:(g + 1) * G, :], sh % S, axis=1)
            valid = (lane >= sh) if sh > 0 else (lane < S + sh)
            hs_sc[g * G:(g + 1) * G, :] = jnp.where(valid, r, 0.0)

        cw0.wait()
        for b in range(2):
            wt_s[b, 0:P0, :] = wqkv_ref[b * D2:(b + 1) * D2, 0:P0].T
        cx0.wait()
        do_q(0)
        cw1.wait()
        for b in range(2):
            wt_s[b, P0:, :] = wqkv_ref[b * D2:(b + 1) * D2, P0:].T
        do_k(0)
        do_v(0)
        cx1.wait()
        c1.wait()
        halves_t(w1_ref[...], w1_s)
        for n in range(7):
            w1_o[n] = _st_lhs(half_blk(w1_s), n)
        for f, c in ((do_k, 1), (do_k, 2), (do_h, 0), (do_v, 1), (do_k, 3), (do_h, 1), (do_v, 2)):
            f(c)
        c3.wait()
        c2.wait()
        co.wait()
        c4.wait()
        do_q(1)
        do_q(2)
        for j in range(4):
            prep_w3(j)
        halves_t(w2_ref[...], w2_s)
        prep_wo()
        do_h(2)
        do_v(3)
        do_h(3)
        for g in range(4):
            shift(g)
        do_q(3)

    q0 = pl.multiple_of(i * TQ, TQ)
    bufs = (sa, sb)

    def masked_q(h):
        g, j = h // 4, h % 4
        lo, hi = (j * DH) // 16 * 16, -(-((j + 1) * DH) // 16) * 16
        qw = q_sc[g * G + lo:g * G + hi, pl.ds(q0, TQ)]
        row = jax.lax.broadcasted_iota(jnp.int32, (hi - lo, TQ), 0) + lo
        qw = jnp.where((row >= j * DH) & (row < (j + 1) * DH), qw, jnp.zeros_like(qw))
        parts = []
        if lo > 0:
            parts.append(jnp.zeros((lo, TQ), bf16))
        parts.append(qw)
        parts.append(jnp.zeros((128 - hi, TQ), bf16))
        return jnp.concatenate(parts, axis=0)

    def qk_chunk(st, c, qm, mpart):
        s = _dot(k_sc[st * HS // 4, c * TK:(c + 1) * TK, :], qm)
        bufs[st % 2][c * TK:(c + 1) * TK, :] = s
        sm = jnp.max(s.reshape(TK // 8, 8, W), axis=0)
        return sm if mpart is None else jnp.maximum(mpart, sm)

    def pv_chunk(st, c, m, acc):
        o = []
        for k in range(HS):
            sl = slice(k * TQ, (k + 1) * TQ)
            p = jnp.exp2(bufs[st % 2][c * TK:(c + 1) * TK, sl] - m[:, sl]).astype(bf16)
            o.append(_dot(vt_sc[st * HS + k, :, c * TK:(c + 1) * TK], p))
        return o if acc is None else [x + y for x, y in zip(acc, o)]

    env = {}

    def do_x1():
        hblk = lambda a, b: hs_sc[a * D2:(a + 1) * D2, pl.ds(pl.multiple_of(q0 + b * T2, T2), T2)]
        m2 = products(lambda n: _st_lhs(half_blk(w2_s), n), lambda n: _st_rhs(hblk, n))
        xf = xt_ref[:, pl.ds(q0, TQ)].astype(f32)
        x1 = xf + 0.5 * _st_join(_st_out(m2))
        x1_sc[...] = x1
        env['m'], env['r'] = _ln_stats(x1)
        gl = jnp.sum(xf * jnp.tile(gwc_sc[...], (1, TQ // 128)), axis=0, keepdims=True)
        env['g'] = jax.nn.sigmoid(gl)

    def do_w3():
        xblk = lambda a, b: x1_sc[a * G:(a + 1) * G, b * T2:(b + 1) * T2]
        mm = [env['m'][:, b * T2:(b + 1) * T2] for b in range(2)]
        rr = [env['r'][:, b * T2:(b + 1) * T2] for b in range(2)]
        m3 = {}
        for n, p in enumerate(_HK):
            m3[p] = _dot(w3_s[n], _hk_rhs_ln(xblk, mm, rr, p))
            fence()
            if p[0] == 'Q':
                j = p[1]
                for b, v in enumerate(_hk_out(m3, j)):
                    hv = _gelu2(v)
                    a, r = divmod(j, 2)
                    hf_sc[a, b, r * 384:(r + 1) * 384, :] = hv[:384]
                    hf_sc[a, b, 768 + r * 64:768 + (r + 1) * 64, :] = hv[384:]
        for n in range(7):
            h3_sc[n] = _st_rhs(lambda a, b: hf_sc[a, b], n)

    m4 = [None] * 7

    def do_w4(n):
        blk = lambda a, b: jnp.concatenate([w4t_ref[a * D2:(a + 1) * D2, b * 768:(b + 1) * 768],
                                            w4t_ref[a * D2:(a + 1) * D2, 1536 + b * 128:1536 + (b + 1) * 128]], axis=1)
        m4[n] = _dot(_st_lhs(blk, n), h3_sc[n])
        fence()

    t_qk = NS * NC
    off = NC + LAG
    extra = {X1_AT: [do_x1], W3_AT: [do_w3]}
    for n in range(7):
        slot = min(t_qk - 1 + n * W4_STEP, t_qk + off - 1)
        extra.setdefault(slot, []).append(functools.partial(do_w4, PORDER[n]))

    ms, mpart, accs, qms = {}, {}, {}, {}
    for t in range(t_qk + off):
        if t < t_qk:
            st, c = divmod(t, NC)
            if c == 0:
                qms[st] = jnp.concatenate([masked_q(st * HS + k) for k in range(HS)], axis=1)
            mpart[st] = qk_chunk(st, c, qms[st], mpart.get(st))
            if c == NC - 1:
                ms[st] = jnp.max(mpart[st], axis=0, keepdims=True)
        u = t - off
        if u >= 0:
            st, c = divmod(u, NC)
            accs[st] = pv_chunk(st, c, ms[st], accs.get(st))
            if c == NC - 1:
                for k in range(HS):
                    acc = accs[st][k]
                    ot_sc[st * HS + k] = acc * (1.0 / acc[DH:DH + 1, :])
        for f in extra.get(t, ()):
            f()

    oblk = lambda a, b: ot_sc[a * (H // 2):(a + 1) * (H // 2), :, b * T2:(b + 1) * T2].reshape(DP // 2, T2)
    mo = products(lambda n: _st_lhs(half_blk(wo_s), n), lambda n: _st_rhs(oblk, n))
    b = x1_sc[...] + 0.5 * _st_join(_st_out(m4))
    a = _st_join(_st_out(mo))
    g = env['g']
    o_ref[...] = (g * a + (1.0 - g) * b).astype(o_ref.dtype)


@jax.jit
def pallas_gated_mix__mha_block__mixer_s_mlp__prompt_kernel(
    A_x: jax.Array,
    A_wqkv: jax.Array,
    A_wo: jax.Array,
    B_x: jax.Array,
    B_w1: jax.Array,
    B_w2: jax.Array,
    B_w3: jax.Array,
    B_w4: jax.Array,
    gate_w: jax.Array,
):
    del B_x
    xt = A_x.reshape(S, D).T
    vm = pltpu.VMEM
    out = pl.pallas_call(
        _kernel,
        grid=(S // TQ,),
        in_specs=[pl.BlockSpec(memory_space=pl.ANY)] * 8,
        out_specs=pl.BlockSpec((D, TQ), lambda i: (0, i)),
        out_shape=jax.ShapeDtypeStruct((D, S), bf16),
        scratch_shapes=[
            vm((D, S), bf16), vm((D, 3 * D), bf16), vm((D, D), bf16), vm((D, D), bf16), vm((D, D), bf16),
            vm((D, F), bf16), vm((D, F), bf16), vm((D,), bf16), pltpu.SemaphoreType.DMA((10,)),
            vm((2, 3 * D, D2), bf16), vm((7, D2, D2), bf16), vm((2, D, D2), bf16), vm((2, D, D2), bf16),
            vm((26, D, G), bf16), vm((2, D, DP // 2), bf16), vm((D, 128), f32),
            vm((D, S), bf16), vm((4, S, 128), bf16), vm((H, HP, S), bf16),
            vm((D, S), f32), vm((D, S), f32), vm((H, HP, TQ), f32),
            vm((7, F2, T2), bf16), vm((2, 2, F2, T2), f32), vm((D, TQ), f32), vm((8, 128), f32),
            vm((S, W), f32), vm((S, W), f32),
        ],
        compiler_params=pltpu.CompilerParams(dimension_semantics=("arbitrary",),
                                             vmem_limit_bytes=100 * 1024 * 1024,
                                             disable_semaphore_checks=True, disable_bounds_checks=True),
        name="gm",
    )(xt, A_wqkv, A_wo, B_w1, B_w2, B_w3, B_w4.T, gate_w)
    return out.T.reshape(1, S, D)
```

```python
import functools

import jax
import jax.numpy as jnp
import jax.experimental.pallas as pl
import jax.experimental.pallas.tpu as pltpu

S, D, H, DH, F = 2048, 448, 16, 28, 1792
HP = 32
DP = H * HP
G = 112
TQ = 256
HS = 2
NS = H // HS
W = TQ * HS
TK = 128
NC = S // TK
CH = 512
LAG = 1
X1_AT, W3_AT, W4_STEP = 1, 12, 4
PORDER = (1, 3, 2, 4, 0, 6, 5)
D2, F2, T2, C2 = D // 2, F // 2, TQ // 2, CH // 2
LOG2E = 1.4426950408889634
EPS = 1e-5
f32, bf16 = jnp.float32, jnp.bfloat16


def _gelu2(x):
    c = 0.7978845608028654
    return x + x * jnp.tanh(x * (c + (c * 0.044715) * (x * x)))


def _ln_stats(x):
    m = jnp.mean(x, axis=0, keepdims=True)
    var = jnp.maximum(jnp.mean(x * x, axis=0, keepdims=True) - m * m, 0.0)
    return m, jax.lax.rsqrt(var + EPS)


def _dot(a, b):
    return jnp.dot(a, b, preferred_element_type=f32)


_LHS = (((0, 0), (1, 1), 1), ((1, 0), (1, 1), 1), ((0, 0), None, 0), ((1, 1), None, 0),
        ((0, 0), (0, 1), 1), ((1, 0), (0, 0), -1), ((0, 1), (1, 1), -1))
_RHS = (((0, 0), (1, 1), 1), ((0, 0), None, 0), ((0, 1), (1, 1), -1), ((1, 0), (0, 0), -1),
        ((1, 1), None, 0), ((0, 0), (0, 1), 1), ((1, 0), (1, 1), 1))


def _st_operand(table, blk, n):
    p, q, sign = table[n]
    if q is None:
        return blk(*p).astype(bf16)
    u, v = blk(*p).astype(f32), blk(*q).astype(f32)
    return (u + v if sign > 0 else u - v).astype(bf16)


_st_lhs = functools.partial(_st_operand, _LHS)
_st_rhs = functools.partial(_st_operand, _RHS)


def _st_out(m):
    return (m[0] + m[3] - m[4] + m[6], m[2] + m[4], m[1] + m[3], m[0] - m[1] + m[2] + m[5])


def _st_join(c):
    return jnp.concatenate([jnp.concatenate(c[:2], axis=1), jnp.concatenate(c[2:], axis=1)], axis=0)


_HT = (0.0, 1.0, -1.0, 2.0)
_HK = []
for _j in range(4):
    _new = [('P', _j, _j), ('Q', _j, _j)]
    for _i in range(_j + 1, 4):
        _new = [('M', _j, _i), ('T', _j, _i), ('T', _i, _j)] + _new
    _HK += _new


def _lin(terms):
    acc = None
    for c, v in sorted([t for t in terms if t[0] != 0.0], key=lambda t: t[0] < 0):
        x = v()
        if abs(c) != 1.0:
            x = x * abs(c)
        if acc is None:
            acc = x if c > 0 else -x
        else:
            acc = acc + x if c > 0 else acc - x
    return acc


def _hk_lhs(blk, p):
    kind, i, j = p
    f = lambda a, b: (lambda: blk(a, b).astype(f32))
    if kind == 'T':
        return blk(j, i).astype(bf16)
    if kind == 'M':
        return _lin([(1.0, f(j, i)), (1.0, f(i, j))]).astype(bf16)
    if kind == 'P':
        return _lin([(1.0 if r == i else -1.0, f(r, i)) for r in range(4)]).astype(bf16)
    return _lin([(1.0, f(i, r)) for r in range(4)]).astype(bf16)


def _hk_rhs_coef(p):
    kind, i, j = p
    if kind == 'P':
        return {i: 1.0}, {}, 1.0
    if kind == 'Q':
        return {i: _HT[i]}, {i: 1.0}, 1.0
    d = _HT[i] - _HT[j]
    sg = 1.0 if d > 0 else -1.0
    if kind == 'M':
        return {i: sg * _HT[i], j: -sg * _HT[j]}, {i: sg, j: -sg}, abs(d)
    return {j: sg * _HT[j], i: -sg * _HT[j]}, {j: sg, i: -sg}, abs(d)


def _hk_rhs_ln(blk, m, r, p):
    c0, c1, d = _hk_rhs_coef(p)
    acc, off = None, None
    for n, c in enumerate((c0, c1)):
        c = {k: v for k, v in c.items() if v != 0.0}
        if not c:
            continue
        g = min(abs(v) for v in c.values())
        if all(v < 0 for v in c.values()):
            g = -g
        rs = r[n] * (g / d)
        x = _lin([(v / g, functools.partial(blk, k, n)) for k, v in c.items()]) * rs
        acc = x if acc is None else acc + x
        tot = sum(c.values()) / g
        if tot != 0.0:
            o = m[n] * rs * tot
            off = o if off is None else off + o
    return (acc if off is None else acc - off).astype(bf16)


def _hk_out(m, j):
    k = lambda v: (lambda: v)
    others = [i for i in range(4) if i != j]
    gjj = _lin([(1.0, k(m['M', min(i, j), max(i, j)])) for i in others] + [(1.0, k(m['T', j, i])) for i in others]
               + [(1.0, k(m['P', j, j]))])
    z0 = _lin([(1.0, k(m['T', i, j])) for i in others] + [(1.0, k(gjj))])
    z1 = _lin([(1.0, k(m['Q', j, j]))] + [(-_HT[i], k(m['T', i, j])) for i in others] + [(-_HT[j], k(gjj))])
    return z0, z1


def _kernel(xt_hbm, wqkv_hbm, wo_hbm, w1_hbm, w2_hbm, w3_hbm, w4t_hbm, gw_hbm,
            o_ref,
            xt_ref, wqkv_ref, wo_ref, w1_ref, w2_ref, w3_ref, w4t_ref, gw_ref, sems,
            wt_s, w1_o, w1_s, w2_s, w3_s, wo_s, gwc_sc,
            q_sc, k_sc, vt_sc, h_sc, hs_sc, ot_sc, h3_sc, hf_sc, x1_sc, fz_sc, sa, sb):
    i = pl.program_id(0)
    half_blk = lambda r: (lambda a, b: r[b, a * D2:(a + 1) * D2, :])

    def fence():
        fz_sc[...] = jnp.zeros((8, 128), f32)

    def products(lhs, rhs):
        m = [None] * 7
        for n in PORDER:
            m[n] = _dot(lhs(n), rhs(n))
            fence()
        return m

    @pl.when(i == 0)
    def _():
        def cp(src, dst, n):
            return pltpu.make_async_copy(src, dst, sems.at[n])
        wpiece = lambda a, b, n: cp(wqkv_hbm.at[:, a:b], wqkv_ref.at[:, a:b], n)
        xpiece = lambda a, b, n: cp(xt_hbm.at[:, a:b], xt_ref.at[:, a:b], n)
        cwk, cwq, cwv = wpiece(384, 2 * D, 0), wpiece(0, 384, 1), wpiece(2 * D, 3 * D, 10)
        cxa, cxb, cx1, cx2 = xpiece(0, C2, 2), xpiece(C2, CH, 11), xpiece(CH, 2 * CH, 3), xpiece(2 * CH, S, 12)
        c1, c2, c3, c4, co, cg = (cp(w1_hbm, w1_ref, 4), cp(w2_hbm, w2_ref, 5), cp(w3_hbm, w3_ref, 6),
                                  cp(w4t_hbm, w4t_ref, 7), cp(wo_hbm, wo_ref, 8), cp(gw_hbm, gw_ref, 9))
        for c in (cg, cwk, cxa, cxb, cwq, cwv, cx1, c1, cx2, c3, c2, co, c4):
            c.start()
        sa[0:8, :] = jnp.zeros((8, W), f32)
        x1_sc[0:8, :] = jnp.zeros((8, TQ), f32)
        hf_sc[0, 0, 0:8, :] = jnp.zeros((8, T2), f32)
        sb[0:8, :] = jnp.zeros((8, W), f32)
        cg.wait()
        gwc_sc[...] = jnp.broadcast_to(gw_ref[...].astype(f32).reshape(1, D), (128, D)).T

        z16 = jnp.zeros((128 - G, CH), bf16)
        tail = jnp.where(jax.lax.broadcasted_iota(jnp.int32, (HP - DH, CH), 0) == 0, 1.0, 0.0).astype(f32)
        chunk = lambda c: slice(c * CH, (c + 1) * CH)
        never = jax.lax.broadcasted_iota(jnp.int32, (D, CH), 1) < i
        stats = {}

        def proj(w, c, fast):
            if not fast:
                return (_dot(wt_s[0, w * D:(w + 1) * D, :], xt_ref[0:D2, chunk(c)])
                        + _dot(wt_s[1, w * D:(w + 1) * D, :], xt_ref[D2:, chunk(c)]))
            ablk = lambda a, b: wt_s[b, w * D + a * D2:w * D + (a + 1) * D2, :]
            xblk = lambda a, b: xt_ref[a * D2:(a + 1) * D2, c * CH + b * C2:c * CH + (b + 1) * C2]
            return _st_join(_st_out(products(lambda n: _st_lhs(ablk, n), lambda n: _st_rhs(xblk, n))))

        def do_q(c):
            q_sc[:, chunk(c)] = (proj(0, c, False) * (DH ** -0.5 * LOG2E)).astype(bf16)

        def do_k(c):
            cs = chunk(c)
            kt = proj(1, c, False)
            stats[c] = _ln_stats(jnp.where(never, kt, xt_ref[:, cs].astype(f32)))
            for g in range(4):
                kg = jnp.concatenate([kt[g * G:(g + 1) * G].astype(bf16), z16], axis=0)
                k_sc[g, cs, :] = kg.T

        def do_v(c):
            vt = proj(2, c, True)
            for h in range(H):
                vh = jnp.concatenate([vt[h * DH:(h + 1) * DH], tail], axis=0)
                vt_sc[h, :, chunk(c)] = vh.astype(bf16)

        def do_h(c):
            m, r = stats[c]
            nblk = lambda a, b: ((xt_ref[a * D2:(a + 1) * D2, c * CH + b * C2:c * CH + (b + 1) * C2].astype(f32)
                                  - m[:, b * C2:(b + 1) * C2]) * r[:, b * C2:(b + 1) * C2])
            y = products(lambda n: w1_o[n], lambda n: _st_rhs(nblk, n))
            h_sc[:, chunk(c)] = _gelu2(_st_join(_st_out(y)))

        def prep_w3(j):
            if j < 3:
                blk = lambda r, k: w3_ref[k * G:(k + 1) * G, r * 384 + j * 128:r * 384 + (j + 1) * 128]
                rows = slice(j * 128, (j + 1) * 128)
            else:
                blk = lambda r, k: w3_ref[k * G:(k + 1) * G, 1536 + r * 64:1536 + (r + 1) * 64]
                rows = slice(384, D)
            for n, p in enumerate(_HK):
                w3_s[n, rows, :] = _hk_lhs(blk, p).T

        def halves_t(w, dst):
            k2 = w.shape[0] // 2
            dst[0] = w[:k2].T
            dst[1] = w[k2:].T

        def prep_wo():
            wo = wo_ref[...].astype(f32)
            z4 = jnp.zeros((HP - DH, D), f32)
            wop = jnp.concatenate([p for h in range(H) for p in (wo[h * DH:(h + 1) * DH], z4)], axis=0)
            halves_t(wop.astype(bf16), wo_s)

        def shift(g):
            sh = (1, -1, 2, -2)[g]
            lane = jax.lax.broadcasted_iota(jnp.int32, (G, S), 1)
            r = pltpu.roll(h_sc[g * G:(g + 1) * G, :], sh % S, axis=1)
            valid = (lane >= sh) if sh > 0 else (lane < S + sh)
            hs_sc[g * G:(g + 1) * G, :] = jnp.where(valid, r, 0.0)

        def wt(a, b):
            for k in range(2):
                wt_s[k, a:b, :] = wqkv_ref[k * D2:(k + 1) * D2, a:b].T

        def k_half(b):
            cs = slice(b * C2, (b + 1) * C2)
            kt = _dot(wt_s[0, D:2 * D, :], xt_ref[0:D2, cs]) + _dot(wt_s[1, D:2 * D, :], xt_ref[D2:, cs])
            st = _ln_stats(jnp.where(jax.lax.broadcasted_iota(jnp.int32, (D, C2), 1) < i, kt, xt_ref[:, cs].astype(f32)))
            return kt.astype(bf16), st

        cwk.wait()
        wt(384, 640)
        cxa.wait()
        wt(640, 2 * D)
        ka, sta = k_half(0)
        cxb.wait()
        cwq.wait()
        wt(0, 384)
        kb, stb = k_half(1)
        stats[0] = tuple(jnp.concatenate([u, v], axis=1) for u, v in zip(sta, stb))
        k0 = jnp.concatenate([ka, kb], axis=1)
        for g in range(4):
            k_sc[g, 0:CH, :] = jnp.concatenate([k0[g * G:(g + 1) * G], z16], axis=0).T
        do_q(0)
        cwv.wait()
        cx1.wait()
        c1.wait()
        wt(2 * D, 3 * D)
        halves_t(w1_ref[...], w1_s)
        for n in range(7):
            w1_o[n] = _st_lhs(half_blk(w1_s), n)
        for f, c in ((do_k, 1), (do_v, 0), (do_h, 0), (do_v, 1), (do_h, 1)):
            f(c)
        cx2.wait()
        c3.wait()
        c2.wait()
        co.wait()
        for f, c in ((do_k, 2), (do_q, 1), (do_q, 2), (do_q, 3)):
            f(c)
        for j in range(4):
            prep_w3(j)
        halves_t(w2_ref[...], w2_s)
        prep_wo()
        for f, c in ((do_h, 2), (do_k, 3), (do_v, 2), (do_h, 3)):
            f(c)
        for g in range(4):
            shift(g)
        do_v(3)
        c4.wait()

    q0 = pl.multiple_of(i * TQ, TQ)
    bufs = (sa, sb)

    def masked_q(h):
        g, j = h // 4, h % 4
        lo, hi = (j * DH) // 16 * 16, -(-((j + 1) * DH) // 16) * 16
        qw = q_sc[g * G + lo:g * G + hi, pl.ds(q0, TQ)]
        row = jax.lax.broadcasted_iota(jnp.int32, (hi - lo, TQ), 0) + lo
        qw = jnp.where((row >= j * DH) & (row < (j + 1) * DH), qw, jnp.zeros_like(qw))
        parts = []
        if lo > 0:
            parts.append(jnp.zeros((lo, TQ), bf16))
        parts.append(qw)
        parts.append(jnp.zeros((128 - hi, TQ), bf16))
        return jnp.concatenate(parts, axis=0)

    def qk_chunk(st, c, qm, mpart):
        s = _dot(k_sc[st * HS // 4, c * TK:(c + 1) * TK, :], qm)
        bufs[st % 2][c * TK:(c + 1) * TK, :] = s
        sm = jnp.max(s.reshape(TK // 8, 8, W), axis=0)
        return sm if mpart is None else jnp.maximum(mpart, sm)

    def pv_chunk(st, c, m, acc):
        o = []
        for k in range(HS):
            sl = slice(k * TQ, (k + 1) * TQ)
            p = jnp.exp2(bufs[st % 2][c * TK:(c + 1) * TK, sl] - m[:, sl]).astype(bf16)
            o.append(_dot(vt_sc[st * HS + k, :, c * TK:(c + 1) * TK], p))
        return o if acc is None else [x + y for x, y in zip(acc, o)]

    env = {}

    def do_x1():
        hblk = lambda a, b: hs_sc[a * D2:(a + 1) * D2, pl.ds(pl.multiple_of(q0 + b * T2, T2), T2)]
        m2 = products(lambda n: _st_lhs(half_blk(w2_s), n), lambda n: _st_rhs(hblk, n))
        xf = xt_ref[:, pl.ds(q0, TQ)].astype(f32)
        x1 = xf + 0.5 * _st_join(_st_out(m2))
        x1_sc[...] = x1
        env['m'], env['r'] = _ln_stats(x1)
        gl = jnp.sum(xf * jnp.tile(gwc_sc[...], (1, TQ // 128)), axis=0, keepdims=True)
        env['g'] = jax.nn.sigmoid(gl)

    def do_w3():
        xblk = lambda a, b: x1_sc[a * G:(a + 1) * G, b * T2:(b + 1) * T2]
        mm = [env['m'][:, b * T2:(b + 1) * T2] for b in range(2)]
        rr = [env['r'][:, b * T2:(b + 1) * T2] for b in range(2)]
        m3 = {}
        for n, p in enumerate(_HK):
            m3[p] = _dot(w3_s[n], _hk_rhs_ln(xblk, mm, rr, p))
            fence()
            if p[0] == 'Q':
                j = p[1]
                for b, v in enumerate(_hk_out(m3, j)):
                    hv = _gelu2(v)
                    a, r = divmod(j, 2)
                    hf_sc[a, b, r * 384:(r + 1) * 384, :] = hv[:384]
                    hf_sc[a, b, 768 + r * 64:768 + (r + 1) * 64, :] = hv[384:]
        for n in range(7):
            h3_sc[n] = _st_rhs(lambda a, b: hf_sc[a, b], n)

    m4 = [None] * 7

    def do_w4(n):
        blk = lambda a, b: jnp.concatenate([w4t_ref[a * D2:(a + 1) * D2, b * 768:(b + 1) * 768],
                                            w4t_ref[a * D2:(a + 1) * D2, 1536 + b * 128:1536 + (b + 1) * 128]], axis=1)
        m4[n] = _dot(_st_lhs(blk, n), h3_sc[n])
        fence()

    t_qk = NS * NC
    off = NC + LAG
    extra = {X1_AT: [do_x1], W3_AT: [do_w3]}
    for n in range(7):
        slot = min(t_qk - 1 + n * W4_STEP, t_qk + off - 1)
        extra.setdefault(slot, []).append(functools.partial(do_w4, PORDER[n]))

    ms, mpart, accs, qms = {}, {}, {}, {}
    for t in range(t_qk + off):
        if t < t_qk:
            st, c = divmod(t, NC)
            if c == 0:
                qms[st] = jnp.concatenate([masked_q(st * HS + k) for k in range(HS)], axis=1)
            mpart[st] = qk_chunk(st, c, qms[st], mpart.get(st))
            if c == NC - 1:
                ms[st] = jnp.max(mpart[st], axis=0, keepdims=True)
        u = t - off
        if u >= 0:
            st, c = divmod(u, NC)
            accs[st] = pv_chunk(st, c, ms[st], accs.get(st))
            if c == NC - 1:
                for k in range(HS):
                    acc = accs[st][k]
                    ot_sc[st * HS + k] = acc * (1.0 / acc[DH:DH + 1, :])
        for f in extra.get(t, ()):
            f()

    oblk = lambda a, b: ot_sc[a * (H // 2):(a + 1) * (H // 2), :, b * T2:(b + 1) * T2].reshape(DP // 2, T2)
    mo = products(lambda n: _st_lhs(half_blk(wo_s), n), lambda n: _st_rhs(oblk, n))
    b = x1_sc[...] + 0.5 * _st_join(_st_out(m4))
    a = _st_join(_st_out(mo))
    g = env['g']
    o_ref[...] = (g * a + (1.0 - g) * b).astype(o_ref.dtype)


@jax.jit
def pallas_gated_mix__mha_block__mixer_s_mlp__prompt_kernel(
    A_x: jax.Array,
    A_wqkv: jax.Array,
    A_wo: jax.Array,
    B_x: jax.Array,
    B_w1: jax.Array,
    B_w2: jax.Array,
    B_w3: jax.Array,
    B_w4: jax.Array,
    gate_w: jax.Array,
):
    del B_x
    xt = A_x.reshape(S, D).T
    vm = pltpu.VMEM
    out = pl.pallas_call(
        _kernel,
        grid=(S // TQ,),
        in_specs=[pl.BlockSpec(memory_space=pl.ANY)] * 8,
        out_specs=pl.BlockSpec((D, TQ), lambda i: (0, i)),
        out_shape=jax.ShapeDtypeStruct((D, S), bf16),
        scratch_shapes=[
            vm((D, S), bf16), vm((D, 3 * D), bf16), vm((D, D), bf16), vm((D, D), bf16), vm((D, D), bf16),
            vm((D, F), bf16), vm((D, F), bf16), vm((D,), bf16), pltpu.SemaphoreType.DMA((13,)),
            vm((2, 3 * D, D2), bf16), vm((7, D2, D2), bf16), vm((2, D, D2), bf16), vm((2, D, D2), bf16),
            vm((26, D, G), bf16), vm((2, D, DP // 2), bf16), vm((D, 128), f32),
            vm((D, S), bf16), vm((4, S, 128), bf16), vm((H, HP, S), bf16),
            vm((D, S), f32), vm((D, S), f32), vm((H, HP, TQ), f32),
            vm((7, F2, T2), bf16), vm((2, 2, F2, T2), f32), vm((D, TQ), f32), vm((8, 128), f32),
            vm((S, W), f32), vm((S, W), f32),
        ],
        compiler_params=pltpu.CompilerParams(dimension_semantics=("arbitrary",),
                                             vmem_limit_bytes=100 * 1024 * 1024,
                                             disable_semaphore_checks=True, disable_bounds_checks=True),
        name="gm",
    )(xt, A_wqkv, A_wo, B_w1, B_w2, B_w3, B_w4.T, gate_w)
    return out.T.reshape(1, S, D)
```

```python
import functools

import jax
import jax.numpy as jnp
import jax.experimental.pallas as pl
import jax.experimental.pallas.tpu as pltpu

S, D, H, DH, F = 2048, 448, 16, 28, 1792
HP = 32
DP = H * HP
G = 112
TQ = 256
HS = 2
NS = H // HS
W = TQ * HS
TK = 128
NC = S // TK
CH = 512
LAG = 1
X1_AT, W3_AT, W4_STEP = 1, 12, 4
PORDER = (1, 3, 2, 4, 0, 6, 5)
D2, F2, T2, C2 = D // 2, F // 2, TQ // 2, CH // 2
LOG2E = 1.4426950408889634
EPS = 1e-5
f32, bf16 = jnp.float32, jnp.bfloat16


def _gelu2(x):
    c = 0.7978845608028654
    return x + x * jnp.tanh(x * (c + (c * 0.044715) * (x * x)))


def _ln_stats(x):
    m = jnp.mean(x, axis=0, keepdims=True)
    var = jnp.maximum(jnp.mean(x * x, axis=0, keepdims=True) - m * m, 0.0)
    return m, jax.lax.rsqrt(var + EPS)


def _dot(a, b):
    return jnp.dot(a, b, preferred_element_type=f32)


_LHS = (((0, 0), (1, 1), 1), ((1, 0), (1, 1), 1), ((0, 0), None, 0), ((1, 1), None, 0),
        ((0, 0), (0, 1), 1), ((1, 0), (0, 0), -1), ((0, 1), (1, 1), -1))
_RHS = (((0, 0), (1, 1), 1), ((0, 0), None, 0), ((0, 1), (1, 1), -1), ((1, 0), (0, 0), -1),
        ((1, 1), None, 0), ((0, 0), (0, 1), 1), ((1, 0), (1, 1), 1))


def _st_operand(table, blk, n):
    p, q, sign = table[n]
    if q is None:
        return blk(*p).astype(bf16)
    u, v = blk(*p).astype(f32), blk(*q).astype(f32)
    return (u + v if sign > 0 else u - v).astype(bf16)


_st_lhs = functools.partial(_st_operand, _LHS)
_st_rhs = functools.partial(_st_operand, _RHS)


def _st_out(m):
    return (m[0] + m[3] - m[4] + m[6], m[2] + m[4], m[1] + m[3], m[0] - m[1] + m[2] + m[5])


def _st_join(c):
    return jnp.concatenate([jnp.concatenate(c[:2], axis=1), jnp.concatenate(c[2:], axis=1)], axis=0)


_HT = (0.0, 1.0, -1.0, 2.0)
_HK = []
for _j in range(4):
    _new = [('P', _j, _j), ('Q', _j, _j)]
    for _i in range(_j + 1, 4):
        _new = [('M', _j, _i), ('T', _j, _i), ('T', _i, _j)] + _new
    _HK += _new


def _lin(terms):
    acc = None
    for c, v in sorted([t for t in terms if t[0] != 0.0], key=lambda t: t[0] < 0):
        x = v()
        if abs(c) != 1.0:
            x = x * abs(c)
        if acc is None:
            acc = x if c > 0 else -x
        else:
            acc = acc + x if c > 0 else acc - x
    return acc


def _hk_lhs(blk, p):
    kind, i, j = p
    f = lambda a, b: (lambda: blk(a, b).astype(f32))
    if kind == 'T':
        return blk(j, i).astype(bf16)
    if kind == 'M':
        return _lin([(1.0, f(j, i)), (1.0, f(i, j))]).astype(bf16)
    if kind == 'P':
        return _lin([(1.0 if r == i else -1.0, f(r, i)) for r in range(4)]).astype(bf16)
    return _lin([(1.0, f(i, r)) for r in range(4)]).astype(bf16)


def _hk_rhs_coef(p):
    kind, i, j = p
    if kind == 'P':
        return {i: 1.0}, {}, 1.0
    if kind == 'Q':
        return {i: _HT[i]}, {i: 1.0}, 1.0
    d = _HT[i] - _HT[j]
    sg = 1.0 if d > 0 else -1.0
    if kind == 'M':
        return {i: sg * _HT[i], j: -sg * _HT[j]}, {i: sg, j: -sg}, abs(d)
    return {j: sg * _HT[j], i: -sg * _HT[j]}, {j: sg, i: -sg}, abs(d)


def _st_rhs_coef(n):
    p, q, sign = _RHS[n]
    c = ({}, {})
    c[p[1]][p[0]] = 1.0
    if q is not None:
        c[q[1]][q[0]] = float(sign)
    return c[0], c[1], 1.0


def _rhs_ln(blk, m, r, coef):
    c0, c1, d = coef
    acc, off = None, None
    for n, c in enumerate((c0, c1)):
        c = {k: v for k, v in c.items() if v != 0.0}
        if not c:
            continue
        g = min(abs(v) for v in c.values())
        if all(v < 0 for v in c.values()):
            g = -g
        rs = r[n] * (g / d)
        x = _lin([(v / g, functools.partial(blk, k, n)) for k, v in c.items()]) * rs
        acc = x if acc is None else acc + x
        tot = sum(c.values()) / g
        if tot != 0.0:
            o = m[n] * rs * tot
            off = o if off is None else off + o
    return (acc if off is None else acc - off).astype(bf16)


def _hk_out(m, j):
    k = lambda v: (lambda: v)
    others = [i for i in range(4) if i != j]
    gjj = _lin([(1.0, k(m['M', min(i, j), max(i, j)])) for i in others] + [(1.0, k(m['T', j, i])) for i in others]
               + [(1.0, k(m['P', j, j]))])
    z0 = _lin([(1.0, k(m['T', i, j])) for i in others] + [(1.0, k(gjj))])
    z1 = _lin([(1.0, k(m['Q', j, j]))] + [(-_HT[i], k(m['T', i, j])) for i in others] + [(-_HT[j], k(gjj))])
    return z0, z1


def _pad_heads(v, fill):
    row = jax.lax.broadcasted_iota(jnp.int32, (8, v.shape[1]), 0)
    out = []
    for h in range(H):
        if h % 2 == 0:
            o = h * DH
            edge = jnp.where(row < 4, v[o + 24:o + 32], jnp.where(row == 4, fill, 0.0))
            out.append(jnp.concatenate([v[o:o + 24], edge], axis=0))
        else:
            o = h * DH - 4
            edge = jnp.where(row >= 4, v[o:o + 8], jnp.where(row == 0, fill, 0.0))
            out.append(jnp.concatenate([edge, v[o + 8:o + 32]], axis=0))
    return out


def _kernel(xt_hbm, wqkv_hbm, wo_hbm, w1_hbm, w2_hbm, w3_hbm, w4t_hbm, gw_hbm,
            o_ref,
            xt_ref, wqkv_ref, wo_ref, w1_ref, w2_ref, w3_ref, w4t_ref, gw_ref, sems,
            wt_s, w1_o, w1_s, w2_s, w3_s, wo_s, gwc_sc,
            q_sc, k_sc, vt_sc, h_sc, hs_sc, ot_sc, h3_sc, hf_sc, x1_sc, fz_sc, sa, sb):
    i = pl.program_id(0)
    half_blk = lambda r: (lambda a, b: r[b, a * D2:(a + 1) * D2, :])

    def fence():
        fz_sc[...] = jnp.zeros((8, 128), f32)

    def products(lhs, rhs):
        m = [None] * 7
        for n in PORDER:
            m[n] = _dot(lhs(n), rhs(n))
            fence()
        return m

    @pl.when(i == 0)
    def _():
        def cp(src, dst, n):
            return pltpu.make_async_copy(src, dst, sems.at[n])
        wpiece = lambda a, b, n: cp(wqkv_hbm.at[:, a:b], wqkv_ref.at[:, a:b], n)
        xpiece = lambda a, b, n: cp(xt_hbm.at[:, a:b], xt_ref.at[:, a:b], n)
        cwk, cwq, cwv = wpiece(384, 2 * D, 0), wpiece(0, 384, 1), wpiece(2 * D, 3 * D, 10)
        cxa, cxb, cx1, cx2 = xpiece(0, C2, 2), xpiece(C2, CH, 11), xpiece(CH, 2 * CH, 3), xpiece(2 * CH, S, 12)
        c1, c2, c3, c4, co, cg = (cp(w1_hbm, w1_ref, 4), cp(w2_hbm, w2_ref, 5), cp(w3_hbm, w3_ref, 6),
                                  cp(w4t_hbm, w4t_ref, 7), cp(wo_hbm, wo_ref, 8), cp(gw_hbm, gw_ref, 9))
        for c in (cg, cwk, cxa, cxb, cwq, cwv, cx1, c1, cx2, c3, c2, co, c4):
            c.start()
        sa[0:8, :] = jnp.zeros((8, W), f32)
        x1_sc[0:8, :] = jnp.zeros((8, TQ), f32)
        hf_sc[0, 0, 0:8, :] = jnp.zeros((8, T2), f32)
        sb[0:8, :] = jnp.zeros((8, W), f32)
        cg.wait()
        gwc_sc[...] = jnp.broadcast_to(gw_ref[...].astype(f32).reshape(1, D), (128, D)).T

        z16 = jnp.zeros((128 - G, CH), bf16)
        chunk = lambda c: slice(c * CH, (c + 1) * CH)
        never = jax.lax.broadcasted_iota(jnp.int32, (D, CH), 1) < i
        stats = {}

        def proj(w, c, fast):
            if not fast:
                return (_dot(wt_s[0, w * D:(w + 1) * D, :], xt_ref[0:D2, chunk(c)])
                        + _dot(wt_s[1, w * D:(w + 1) * D, :], xt_ref[D2:, chunk(c)]))
            ablk = lambda a, b: wt_s[b, w * D + a * D2:w * D + (a + 1) * D2, :]
            xblk = lambda a, b: xt_ref[a * D2:(a + 1) * D2, c * CH + b * C2:c * CH + (b + 1) * C2]
            return _st_join(_st_out(products(lambda n: _st_lhs(ablk, n), lambda n: _st_rhs(xblk, n))))

        def do_q(c):
            q_sc[:, chunk(c)] = (proj(0, c, False) * (DH ** -0.5 * LOG2E)).astype(bf16)

        def do_k(c):
            cs = chunk(c)
            kt = proj(1, c, False)
            stats[c] = _ln_stats(jnp.where(never, kt, xt_ref[:, cs].astype(f32)))
            for g in range(4):
                kg = jnp.concatenate([kt[g * G:(g + 1) * G].astype(bf16), z16], axis=0)
                k_sc[g, cs, :] = kg.T

        def do_v(c):
            vt = proj(2, c, True)
            for h, vh in enumerate(_pad_heads(vt, 1.0)):
                vt_sc[h, :, chunk(c)] = vh.astype(bf16)

        def do_h(c):
            m, r = ([v[:, b * C2:(b + 1) * C2] for b in range(2)] for v in stats[c])
            xblk = lambda a, b: xt_ref[a * D2:(a + 1) * D2, c * CH + b * C2:c * CH + (b + 1) * C2].astype(f32)
            y = products(lambda n: w1_o[n], lambda n: _rhs_ln(xblk, m, r, _st_rhs_coef(n)))
            h_sc[:, chunk(c)] = _gelu2(_st_join(_st_out(y)))

        def prep_w3(j):
            if j < 3:
                blk = lambda r, k: w3_ref[k * G:(k + 1) * G, r * 384 + j * 128:r * 384 + (j + 1) * 128]
                rows = slice(j * 128, (j + 1) * 128)
            else:
                blk = lambda r, k: w3_ref[k * G:(k + 1) * G, 1536 + r * 64:1536 + (r + 1) * 64]
                rows = slice(384, D)
            for n, p in enumerate(_HK):
                w3_s[n, rows, :] = _hk_lhs(blk, p).T

        def halves_t(w, dst):
            k2 = w.shape[0] // 2
            dst[0] = w[:k2].T
            dst[1] = w[k2:].T

        def prep_wo():
            wop = jnp.concatenate(_pad_heads(wo_ref[...].astype(f32), 0.0), axis=0)
            halves_t(wop.astype(bf16), wo_s)

        def shift(g):
            sh = (1, -1, 2, -2)[g]
            lane = jax.lax.broadcasted_iota(jnp.int32, (G, S), 1)
            r = pltpu.roll(h_sc[g * G:(g + 1) * G, :], sh % S, axis=1)
            valid = (lane >= sh) if sh > 0 else (lane < S + sh)
            hs_sc[g * G:(g + 1) * G, :] = jnp.where(valid, r, 0.0)

        def wt(a, b):
            for k in range(2):
                wt_s[k, a:b, :] = wqkv_ref[k * D2:(k + 1) * D2, a:b].T

        def k_half(b):
            cs = slice(b * C2, (b + 1) * C2)
            kt = _dot(wt_s[0, D:2 * D, :], xt_ref[0:D2, cs]) + _dot(wt_s[1, D:2 * D, :], xt_ref[D2:, cs])
            st = _ln_stats(jnp.where(jax.lax.broadcasted_iota(jnp.int32, (D, C2), 1) < i, kt, xt_ref[:, cs].astype(f32)))
            return kt.astype(bf16), st

        cwk.wait()
        wt(384, 640)
        cxa.wait()
        wt(640, 2 * D)
        ka, sta = k_half(0)
        cxb.wait()
        cwq.wait()
        wt(0, 384)
        kb, stb = k_half(1)
        stats[0] = tuple(jnp.concatenate([u, v], axis=1) for u, v in zip(sta, stb))
        k0 = jnp.concatenate([ka, kb], axis=1)
        for g in range(4):
            k_sc[g, 0:CH, :] = jnp.concatenate([k0[g * G:(g + 1) * G], z16], axis=0).T
        do_q(0)
        cwv.wait()
        cx1.wait()
        c1.wait()
        wt(2 * D, 3 * D)
        halves_t(w1_ref[...], w1_s)
        for n in range(7):
            w1_o[n] = _st_lhs(half_blk(w1_s), n)
        for f, c in ((do_k, 1), (do_v, 0), (do_h, 0), (do_h, 1), (do_v, 1)):
            f(c)
        cx2.wait()
        c3.wait()
        c2.wait()
        co.wait()
        for f, c in ((do_k, 2), (do_k, 3), (do_q, 1), (do_q, 2)):
            f(c)
        for j in range(4):
            prep_w3(j)
        halves_t(w2_ref[...], w2_s)
        prep_wo()
        for f, c in ((do_h, 2), (do_q, 3), (do_h, 3)):
            f(c)
        for g in range(4):
            shift(g)
        do_v(2)
        do_v(3)
        c4.wait()

    q0 = pl.multiple_of(i * TQ, TQ)
    bufs = (sa, sb)

    def masked_q(h):
        g, j = h // 4, h % 4
        lo, hi = (j * DH) // 16 * 16, -(-((j + 1) * DH) // 16) * 16
        qw = q_sc[g * G + lo:g * G + hi, pl.ds(q0, TQ)]
        row = jax.lax.broadcasted_iota(jnp.int32, (hi - lo, TQ), 0) + lo
        qw = jnp.where((row >= j * DH) & (row < (j + 1) * DH), qw, jnp.zeros_like(qw))
        parts = []
        if lo > 0:
            parts.append(jnp.zeros((lo, TQ), bf16))
        parts.append(qw)
        parts.append(jnp.zeros((128 - hi, TQ), bf16))
        return jnp.concatenate(parts, axis=0)

    def qk_chunk(st, c, qm, mpart):
        s = _dot(k_sc[st * HS // 4, c * TK:(c + 1) * TK, :], qm)
        bufs[st % 2][c * TK:(c + 1) * TK, :] = s
        sm = jnp.max(s.reshape(TK // 8, 8, W), axis=0)
        return sm if mpart is None else jnp.maximum(mpart, sm)

    def pv_chunk(st, c, m, acc):
        o = []
        for k in range(HS):
            sl = slice(k * TQ, (k + 1) * TQ)
            p = jnp.exp2(bufs[st % 2][c * TK:(c + 1) * TK, sl] - m[:, sl]).astype(bf16)
            o.append(_dot(vt_sc[st * HS + k, :, c * TK:(c + 1) * TK], p))
        return o if acc is None else [x + y for x, y in zip(acc, o)]

    env = {}

    def do_x1():
        hblk = lambda a, b: hs_sc[a * D2:(a + 1) * D2, pl.ds(pl.multiple_of(q0 + b * T2, T2), T2)]
        m2 = products(lambda n: _st_lhs(half_blk(w2_s), n), lambda n: _st_rhs(hblk, n))
        xf = xt_ref[:, pl.ds(q0, TQ)].astype(f32)
        x1 = xf + 0.5 * _st_join(_st_out(m2))
        x1_sc[...] = x1
        env['m'], env['r'] = _ln_stats(x1)
        gl = jnp.sum(xf * jnp.tile(gwc_sc[...], (1, TQ // 128)), axis=0, keepdims=True)
        env['g'] = jax.nn.sigmoid(gl)

    def do_w3():
        xblk = lambda a, b: x1_sc[a * G:(a + 1) * G, b * T2:(b + 1) * T2]
        mm = [env['m'][:, b * T2:(b + 1) * T2] for b in range(2)]
        rr = [env['r'][:, b * T2:(b + 1) * T2] for b in range(2)]
        m3 = {}
        for n, p in enumerate(_HK):
            m3[p] = _dot(w3_s[n], _rhs_ln(xblk, mm, rr, _hk_rhs_coef(p)))
            fence()
            if p[0] == 'Q':
                j = p[1]
                for b, v in enumerate(_hk_out(m3, j)):
                    hv = _gelu2(v)
                    a, r = divmod(j, 2)
                    hf_sc[a, b, r * 384:(r + 1) * 384, :] = hv[:384]
                    hf_sc[a, b, 768 + r * 64:768 + (r + 1) * 64, :] = hv[384:]
        for n in range(7):
            h3_sc[n] = _st_rhs(lambda a, b: hf_sc[a, b], n)

    m4 = [None] * 7

    def do_w4(n):
        blk1 = lambda a, b: w4t_ref[a * D2:(a + 1) * D2, b * 768:(b + 1) * 768]
        blk2 = lambda a, b: w4t_ref[a * D2:(a + 1) * D2, 1536 + b * 128:1536 + (b + 1) * 128]
        m4[n] = _dot(_st_lhs(blk1, n), h3_sc[n, 0:768, :]) + _dot(_st_lhs(blk2, n), h3_sc[n, 768:, :])
        fence()

    t_qk = NS * NC
    off = NC + LAG
    extra = {X1_AT: [do_x1], W3_AT: [do_w3]}
    for n in range(7):
        slot = min(t_qk - 1 + n * W4_STEP, t_qk + off - 1)
        extra.setdefault(slot, []).append(functools.partial(do_w4, PORDER[n]))

    ms, mpart, accs, qms = {}, {}, {}, {}
    for t in range(t_qk + off):
        if t < t_qk:
            st, c = divmod(t, NC)
            if c == 0:
                qms[st] = jnp.concatenate([masked_q(st * HS + k) for k in range(HS)], axis=1)
            mpart[st] = qk_chunk(st, c, qms[st], mpart.get(st))
            if c == NC - 1:
                ms[st] = jnp.max(mpart[st], axis=0, keepdims=True)
        u = t - off
        if u >= 0:
            st, c = divmod(u, NC)
            accs[st] = pv_chunk(st, c, ms[st], accs.get(st))
            if c == NC - 1:
                for k in range(HS):
                    acc = accs[st][k]
                    lrow = DH if (st * HS + k) % 2 == 0 else 0
                    ot_sc[st * HS + k] = acc * (1.0 / acc[lrow:lrow + 1, :])
        for f in extra.get(t, ()):
            f()

    oblk = lambda a, b: ot_sc[a * (H // 2):(a + 1) * (H // 2), :, b * T2:(b + 1) * T2].reshape(DP // 2, T2)
    mo = products(lambda n: _st_lhs(half_blk(wo_s), n), lambda n: _st_rhs(oblk, n))
    b = x1_sc[...] + 0.5 * _st_join(_st_out(m4))
    a = _st_join(_st_out(mo))
    g = env['g']
    o_ref[...] = (g * a + (1.0 - g) * b).astype(o_ref.dtype)


@jax.jit
def pallas_gated_mix__mha_block__mixer_s_mlp__prompt_kernel(
    A_x: jax.Array,
    A_wqkv: jax.Array,
    A_wo: jax.Array,
    B_x: jax.Array,
    B_w1: jax.Array,
    B_w2: jax.Array,
    B_w3: jax.Array,
    B_w4: jax.Array,
    gate_w: jax.Array,
):
    del B_x
    xt = A_x.reshape(S, D).T
    vm = pltpu.VMEM
    out = pl.pallas_call(
        _kernel,
        grid=(S // TQ,),
        in_specs=[pl.BlockSpec(memory_space=pl.ANY)] * 8,
        out_specs=pl.BlockSpec((D, TQ), lambda i: (0, i)),
        out_shape=jax.ShapeDtypeStruct((D, S), bf16),
        scratch_shapes=[
            vm((D, S), bf16), vm((D, 3 * D), bf16), vm((D, D), bf16), vm((D, D), bf16), vm((D, D), bf16),
            vm((D, F), bf16), vm((D, F), bf16), vm((D,), bf16), pltpu.SemaphoreType.DMA((13,)),
            vm((2, 3 * D, D2), bf16), vm((7, D2, D2), bf16), vm((2, D, D2), bf16), vm((2, D, D2), bf16),
            vm((26, D, G), bf16), vm((2, D, DP // 2), bf16), vm((D, 128), f32),
            vm((D, S), bf16), vm((4, S, 128), bf16), vm((H, HP, S), bf16),
            vm((D, S), f32), vm((D, S), f32), vm((H, HP, TQ), f32),
            vm((7, F2, T2), bf16), vm((2, 2, F2, T2), f32), vm((D, TQ), f32), vm((8, 128), f32),
            vm((S, W), f32), vm((S, W), f32),
        ],
        compiler_params=pltpu.CompilerParams(dimension_semantics=("arbitrary",),
                                             vmem_limit_bytes=100 * 1024 * 1024,
                                             disable_semaphore_checks=True, disable_bounds_checks=True),
        name="gm",
    )(xt, A_wqkv, A_wo, B_w1, B_w2, B_w3, B_w4.T, gate_w)
    return out.T.reshape(1, S, D)
```

```python
import functools

import jax
import jax.numpy as jnp
import jax.experimental.pallas as pl
import jax.experimental.pallas.tpu as pltpu

S, D, H, DH, F = 2048, 448, 16, 28, 1792
HP = 32
DP = H * HP
G = 112
TQ = 256
HS = 2
NS = H // HS
W = TQ * HS
TK = 128
NC = S // TK
CH = 512
LAG = 1
X1_AT, W3_AT, W4_STEP = 1, 12, 4
PORDER = (1, 3, 2, 4, 0, 6, 5)
D2, F2, T2, C2 = D // 2, F // 2, TQ // 2, CH // 2
LOG2E = 1.4426950408889634
EPS = 1e-5
f32, bf16 = jnp.float32, jnp.bfloat16


def _gelu2(x):
    c = 0.7978845608028654
    return x + x * jnp.tanh(x * (c + (c * 0.044715) * (x * x)))


def _ln_stats(x):
    m = jnp.mean(x, axis=0, keepdims=True)
    var = jnp.maximum(jnp.mean(x * x, axis=0, keepdims=True) - m * m, 0.0)
    return m, jax.lax.rsqrt(var + EPS)


def _dot(a, b):
    return jnp.dot(a, b, preferred_element_type=f32)


_LHS = (((0, 0), (1, 1), 1), ((1, 0), (1, 1), 1), ((0, 0), None, 0), ((1, 1), None, 0),
        ((0, 0), (0, 1), 1), ((1, 0), (0, 0), -1), ((0, 1), (1, 1), -1))
_RHS = (((0, 0), (1, 1), 1), ((0, 0), None, 0), ((0, 1), (1, 1), -1), ((1, 0), (0, 0), -1),
        ((1, 1), None, 0), ((0, 0), (0, 1), 1), ((1, 0), (1, 1), 1))


def _st_operand(table, blk, n):
    p, q, sign = table[n]
    if q is None:
        return blk(*p).astype(bf16)
    u, v = blk(*p).astype(f32), blk(*q).astype(f32)
    return (u + v if sign > 0 else u - v).astype(bf16)


_st_lhs = functools.partial(_st_operand, _LHS)
_st_rhs = functools.partial(_st_operand, _RHS)


def _st_out(m):
    return (m[0] + m[3] - m[4] + m[6], m[2] + m[4], m[1] + m[3], m[0] - m[1] + m[2] + m[5])


def _st_join(c):
    return jnp.concatenate([jnp.concatenate(c[:2], axis=1), jnp.concatenate(c[2:], axis=1)], axis=0)


_HT = (0.0, 1.0, -1.0, 2.0)
_HK = []
for _j in range(4):
    _new = [('P', _j, _j), ('Q', _j, _j)]
    for _i in range(_j + 1, 4):
        _new = [('M', _j, _i), ('T', _j, _i), ('T', _i, _j)] + _new
    _HK += _new


def _lin(terms):
    acc = None
    for c, v in sorted([t for t in terms if t[0] != 0.0], key=lambda t: t[0] < 0):
        x = v()
        if abs(c) != 1.0:
            x = x * abs(c)
        if acc is None:
            acc = x if c > 0 else -x
        else:
            acc = acc + x if c > 0 else acc - x
    return acc


def _hk_lhs(blk, p):
    kind, i, j = p
    f = lambda a, b: (lambda: blk(a, b).astype(f32))
    if kind == 'T':
        return blk(j, i).astype(bf16)
    if kind == 'M':
        return _lin([(1.0, f(j, i)), (1.0, f(i, j))]).astype(bf16)
    if kind == 'P':
        return _lin([(1.0 if r == i else -1.0, f(r, i)) for r in range(4)]).astype(bf16)
    return _lin([(1.0, f(i, r)) for r in range(4)]).astype(bf16)


def _hk_rhs_coef(p):
    kind, i, j = p
    if kind == 'P':
        return {i: 1.0}, {}, 1.0
    if kind == 'Q':
        return {i: _HT[i]}, {i: 1.0}, 1.0
    d = _HT[i] - _HT[j]
    sg = 1.0 if d > 0 else -1.0
    if kind == 'M':
        return {i: sg * _HT[i], j: -sg * _HT[j]}, {i: sg, j: -sg}, abs(d)
    return {j: sg * _HT[j], i: -sg * _HT[j]}, {j: sg, i: -sg}, abs(d)


def _st_rhs_coef(n):
    p, q, sign = _RHS[n]
    c = ({}, {})
    c[p[1]][p[0]] = 1.0
    if q is not None:
        c[q[1]][q[0]] = float(sign)
    return c[0], c[1], 1.0


def _rhs_ln(blk, m, r, coef):
    c0, c1, d = coef
    acc, off = None, None
    for n, c in enumerate((c0, c1)):
        c = {k: v for k, v in c.items() if v != 0.0}
        if not c:
            continue
        g = min(abs(v) for v in c.values())
        if all(v < 0 for v in c.values()):
            g = -g
        rs = r[n] * (g / d)
        x = _lin([(v / g, functools.partial(blk, k, n)) for k, v in c.items()]) * rs
        acc = x if acc is None else acc + x
        tot = sum(c.values()) / g
        if tot != 0.0:
            o = m[n] * rs * tot
            off = o if off is None else off + o
    return (acc if off is None else acc - off).astype(bf16)


def _hk_out(m, j):
    k = lambda v: (lambda: v)
    others = [i for i in range(4) if i != j]
    gjj = _lin([(1.0, k(m['M', min(i, j), max(i, j)])) for i in others] + [(1.0, k(m['T', j, i])) for i in others]
               + [(1.0, k(m['P', j, j]))])
    z0 = _lin([(1.0, k(m['T', i, j])) for i in others] + [(1.0, k(gjj))])
    z1 = _lin([(1.0, k(m['Q', j, j]))] + [(-_HT[i], k(m['T', i, j])) for i in others] + [(-_HT[j], k(gjj))])
    return z0, z1


def _pad_heads(v, fill):
    row = jax.lax.broadcasted_iota(jnp.int32, (8, v.shape[1]), 0)
    out = []
    for h in range(H):
        if h % 2 == 0:
            o = h * DH
            edge = jnp.where(row < 4, v[o + 24:o + 32], jnp.where(row == 4, fill, 0.0))
            out.append(jnp.concatenate([v[o:o + 24], edge], axis=0))
        else:
            o = h * DH - 4
            edge = jnp.where(row >= 4, v[o:o + 8], jnp.where(row == 0, fill, 0.0))
            out.append(jnp.concatenate([edge, v[o + 8:o + 32]], axis=0))
    return out


def _kernel(xt_hbm, wqkv_hbm, wo_hbm, w1_hbm, w2_hbm, w3_hbm, w4t_hbm, gw_hbm,
            o_hbm,
            xt_ref, wqkv_ref, wo_ref, w1_ref, w2_ref, w3_ref, w4t_ref, gw_ref, sems,
            wt_s, w1_o, w1_s, w2_s, w3_s, wo_s, gwc_sc,
            q_sc, k_sc, vt_sc, h_sc, hs_sc, ot_sc, h3_sc, hf_sc, x1_sc, fz_sc, sa, sb, o_sc, osem):
    i = pl.program_id(0)
    half_blk = lambda r: (lambda a, b: r[b, a * D2:(a + 1) * D2, :])

    def fence():
        fz_sc[...] = jnp.zeros((8, 128), f32)

    def products(lhs, rhs):
        m = [None] * 7
        for n in PORDER:
            m[n] = _dot(lhs(n), rhs(n))
            fence()
        return m

    @pl.when(i == 0)
    def _():
        def cp(src, dst, n):
            return pltpu.make_async_copy(src, dst, sems.at[n])
        wpiece = lambda a, b, n: cp(wqkv_hbm.at[:, a:b], wqkv_ref.at[:, a:b], n)
        xpiece = lambda a, b, n: cp(xt_hbm.at[:, a:b], xt_ref.at[:, a:b], n)
        cwk, cwq, cwv = wpiece(384, 2 * D, 0), wpiece(0, 384, 1), wpiece(2 * D, 3 * D, 10)
        cxa, cxb, cx1, cx2 = xpiece(0, C2, 2), xpiece(C2, CH, 11), xpiece(CH, 2 * CH, 3), xpiece(2 * CH, S, 12)
        c1, c2, c3, c4, co, cg = (cp(w1_hbm, w1_ref, 4), cp(w2_hbm, w2_ref, 5), cp(w3_hbm, w3_ref, 6),
                                  cp(w4t_hbm, w4t_ref, 7), cp(wo_hbm, wo_ref, 8), cp(gw_hbm, gw_ref, 9))
        for c in (cg, cwk, cxa, cxb, cwq, cwv, cx1, c1, cx2, c3, c2, co, c4):
            c.start()
        sa[0:8, :] = jnp.zeros((8, W), f32)
        x1_sc[0:8, :] = jnp.zeros((8, TQ), f32)
        hf_sc[0, 0, 0:8, :] = jnp.zeros((8, T2), f32)
        sb[0:8, :] = jnp.zeros((8, W), f32)
        cg.wait()
        gwc_sc[...] = jnp.broadcast_to(gw_ref[...].astype(f32).reshape(1, D), (128, D)).T

        z16 = jnp.zeros((128 - G, CH), bf16)
        chunk = lambda c: slice(c * CH, (c + 1) * CH)
        never = jax.lax.broadcasted_iota(jnp.int32, (D, CH), 1) < i
        stats = {}

        def proj(w, c, fast):
            if not fast:
                return (_dot(wt_s[0, w * D:(w + 1) * D, :], xt_ref[0:D2, chunk(c)])
                        + _dot(wt_s[1, w * D:(w + 1) * D, :], xt_ref[D2:, chunk(c)]))
            ablk = lambda a, b: wt_s[b, w * D + a * D2:w * D + (a + 1) * D2, :]
            xblk = lambda a, b: xt_ref[a * D2:(a + 1) * D2, c * CH + b * C2:c * CH + (b + 1) * C2]
            return _st_join(_st_out(products(lambda n: _st_lhs(ablk, n), lambda n: _st_rhs(xblk, n))))

        def do_q(c):
            q_sc[:, chunk(c)] = (proj(0, c, False) * (DH ** -0.5 * LOG2E)).astype(bf16)

        def do_k(c):
            cs = chunk(c)
            kt = proj(1, c, False)
            stats[c] = _ln_stats(jnp.where(never, kt, xt_ref[:, cs].astype(f32)))
            for g in range(4):
                kg = jnp.concatenate([kt[g * G:(g + 1) * G].astype(bf16), z16], axis=0)
                k_sc[g, cs, :] = kg.T

        def do_v(c):
            vt = proj(2, c, True)
            for h, vh in enumerate(_pad_heads(vt, 1.0)):
                vt_sc[h, :, chunk(c)] = vh.astype(bf16)

        def do_h(c):
            m, r = ([v[:, b * C2:(b + 1) * C2] for b in range(2)] for v in stats[c])
            xblk = lambda a, b: xt_ref[a * D2:(a + 1) * D2, c * CH + b * C2:c * CH + (b + 1) * C2].astype(f32)
            y = products(lambda n: w1_o[n], lambda n: _rhs_ln(xblk, m, r, _st_rhs_coef(n)))
            h_sc[:, chunk(c)] = _gelu2(_st_join(_st_out(y)))

        def prep_w3(j):
            if j < 3:
                blk = lambda r, k: w3_ref[k * G:(k + 1) * G, r * 384 + j * 128:r * 384 + (j + 1) * 128]
                rows = slice(j * 128, (j + 1) * 128)
            else:
                blk = lambda r, k: w3_ref[k * G:(k + 1) * G, 1536 + r * 64:1536 + (r + 1) * 64]
                rows = slice(384, D)
            for n, p in enumerate(_HK):
                w3_s[n, rows, :] = _hk_lhs(blk, p).T

        def halves_t(w, dst):
            k2 = w.shape[0] // 2
            dst[0] = w[:k2].T
            dst[1] = w[k2:].T

        def prep_wo():
            wop = jnp.concatenate(_pad_heads(wo_ref[...].astype(f32), 0.0), axis=0)
            halves_t(wop.astype(bf16), wo_s)

        def shift(g):
            sh = (1, -1, 2, -2)[g]
            lane = jax.lax.broadcasted_iota(jnp.int32, (G, S), 1)
            r = pltpu.roll(h_sc[g * G:(g + 1) * G, :], sh % S, axis=1)
            valid = (lane >= sh) if sh > 0 else (lane < S + sh)
            hs_sc[g * G:(g + 1) * G, :] = jnp.where(valid, r, 0.0)

        def wt(a, b):
            for k in range(2):
                wt_s[k, a:b, :] = wqkv_ref[k * D2:(k + 1) * D2, a:b].T

        def k_half(b):
            cs = slice(b * C2, (b + 1) * C2)
            kt = _dot(wt_s[0, D:2 * D, :], xt_ref[0:D2, cs]) + _dot(wt_s[1, D:2 * D, :], xt_ref[D2:, cs])
            st = _ln_stats(jnp.where(jax.lax.broadcasted_iota(jnp.int32, (D, C2), 1) < i, kt, xt_ref[:, cs].astype(f32)))
            return kt.astype(bf16), st

        cwk.wait()
        wt(384, 640)
        cxa.wait()
        wt(640, 2 * D)
        ka, sta = k_half(0)
        cxb.wait()
        cwq.wait()
        wt(0, 384)
        kb, stb = k_half(1)
        stats[0] = tuple(jnp.concatenate([u, v], axis=1) for u, v in zip(sta, stb))
        k0 = jnp.concatenate([ka, kb], axis=1)
        for g in range(4):
            k_sc[g, 0:CH, :] = jnp.concatenate([k0[g * G:(g + 1) * G], z16], axis=0).T
        do_q(0)
        cwv.wait()
        cx1.wait()
        c1.wait()
        wt(2 * D, 3 * D)
        halves_t(w1_ref[...], w1_s)
        for n in range(7):
            w1_o[n] = _st_lhs(half_blk(w1_s), n)
        for f, c in ((do_k, 1), (do_v, 0), (do_h, 0), (do_h, 1), (do_v, 1)):
            f(c)
        cx2.wait()
        c3.wait()
        c2.wait()
        co.wait()
        for f, c in ((do_k, 2), (do_k, 3), (do_q, 1), (do_q, 2)):
            f(c)
        for j in range(4):
            prep_w3(j)
        halves_t(w2_ref[...], w2_s)
        prep_wo()
        for f, c in ((do_h, 2), (do_q, 3), (do_h, 3)):
            f(c)
        for g in range(4):
            shift(g)
        do_v(2)
        do_v(3)
        c4.wait()

    q0 = pl.multiple_of(i * TQ, TQ)
    bufs = (sa, sb)

    def masked_q(h):
        g, j = h // 4, h % 4
        lo, hi = (j * DH) // 16 * 16, -(-((j + 1) * DH) // 16) * 16
        qw = q_sc[g * G + lo:g * G + hi, pl.ds(q0, TQ)]
        row = jax.lax.broadcasted_iota(jnp.int32, (hi - lo, TQ), 0) + lo
        qw = jnp.where((row >= j * DH) & (row < (j + 1) * DH), qw, jnp.zeros_like(qw))
        parts = []
        if lo > 0:
            parts.append(jnp.zeros((lo, TQ), bf16))
        parts.append(qw)
        parts.append(jnp.zeros((128 - hi, TQ), bf16))
        return jnp.concatenate(parts, axis=0)

    def qk_chunk(st, c, qm, mpart):
        s = _dot(k_sc[st * HS // 4, c * TK:(c + 1) * TK, :], qm)
        bufs[st % 2][c * TK:(c + 1) * TK, :] = s
        sm = jnp.max(s.reshape(TK // 8, 8, W), axis=0)
        return sm if mpart is None else jnp.maximum(mpart, sm)

    def pv_chunk(st, c, m, acc):
        o = []
        for k in range(HS):
            sl = slice(k * TQ, (k + 1) * TQ)
            p = jnp.exp2(bufs[st % 2][c * TK:(c + 1) * TK, sl] - m[:, sl]).astype(bf16)
            o.append(_dot(vt_sc[st * HS + k, :, c * TK:(c + 1) * TK], p))
        return o if acc is None else [x + y for x, y in zip(acc, o)]

    env = {}

    def do_x1():
        hblk = lambda a, b: hs_sc[a * D2:(a + 1) * D2, pl.ds(pl.multiple_of(q0 + b * T2, T2), T2)]
        m2 = products(lambda n: _st_lhs(half_blk(w2_s), n), lambda n: _st_rhs(hblk, n))
        xf = xt_ref[:, pl.ds(q0, TQ)].astype(f32)
        x1 = xf + 0.5 * _st_join(_st_out(m2))
        x1_sc[...] = x1
        env['m'], env['r'] = _ln_stats(x1)
        gl = jnp.sum(xf * jnp.tile(gwc_sc[...], (1, TQ // 128)), axis=0, keepdims=True)
        env['g'] = jax.nn.sigmoid(gl)

    def do_w3():
        xblk = lambda a, b: x1_sc[a * G:(a + 1) * G, b * T2:(b + 1) * T2]
        mm = [env['m'][:, b * T2:(b + 1) * T2] for b in range(2)]
        rr = [env['r'][:, b * T2:(b + 1) * T2] for b in range(2)]
        m3 = {}
        for n, p in enumerate(_HK):
            m3[p] = _dot(w3_s[n], _rhs_ln(xblk, mm, rr, _hk_rhs_coef(p)))
            fence()
            if p[0] == 'Q':
                j = p[1]
                for b, v in enumerate(_hk_out(m3, j)):
                    hv = _gelu2(v)
                    a, r = divmod(j, 2)
                    hf_sc[a, b, r * 384:(r + 1) * 384, :] = hv[:384]
                    hf_sc[a, b, 768 + r * 64:768 + (r + 1) * 64, :] = hv[384:]
        for n in range(7):
            h3_sc[n] = _st_rhs(lambda a, b: hf_sc[a, b], n)

    m4 = [None] * 7

    def do_w4(n):
        blk1 = lambda a, b: w4t_ref[a * D2:(a + 1) * D2, b * 768:(b + 1) * 768]
        blk2 = lambda a, b: w4t_ref[a * D2:(a + 1) * D2, 1536 + b * 128:1536 + (b + 1) * 128]
        m4[n] = _dot(_st_lhs(blk1, n), h3_sc[n, 0:768, :]) + _dot(_st_lhs(blk2, n), h3_sc[n, 768:, :])
        fence()

    t_qk = NS * NC
    off = NC + LAG
    extra = {X1_AT: [do_x1], W3_AT: [do_w3]}
    for n in range(7):
        slot = min(t_qk - 1 + n * W4_STEP, t_qk + off - 1)
        extra.setdefault(slot, []).append(functools.partial(do_w4, PORDER[n]))

    ms, mpart, accs, qms = {}, {}, {}, {}
    for t in range(t_qk + off):
        if t < t_qk:
            st, c = divmod(t, NC)
            if c == 0:
                qms[st] = jnp.concatenate([masked_q(st * HS + k) for k in range(HS)], axis=1)
            mpart[st] = qk_chunk(st, c, qms[st], mpart.get(st))
            if c == NC - 1:
                ms[st] = jnp.max(mpart[st], axis=0, keepdims=True)
        u = t - off
        if u >= 0:
            st, c = divmod(u, NC)
            accs[st] = pv_chunk(st, c, ms[st], accs.get(st))
            if c == NC - 1:
                for k in range(HS):
                    acc = accs[st][k]
                    lrow = DH if (st * HS + k) % 2 == 0 else 0
                    ot_sc[st * HS + k] = acc * (1.0 / acc[lrow:lrow + 1, :])
        for f in extra.get(t, ()):
            f()

    oblk = lambda a, b: ot_sc[a * (H // 2):(a + 1) * (H // 2), :, b * T2:(b + 1) * T2].reshape(DP // 2, T2)
    yb = _st_out(m4)
    g = env['g']
    mo = [None] * 7

    def finish(hf, top, bot):
        sl = slice(hf * T2, (hf + 1) * T2)
        a = jnp.concatenate([top, bot], axis=0)
        b = x1_sc[:, sl] + 0.5 * jnp.concatenate([yb[hf], yb[2 + hf]], axis=0)
        o_sc[i, hf] = (g[:, sl] * a + (1.0 - g[:, sl]) * b).astype(bf16)
        pltpu.make_async_copy(o_sc.at[i, hf], o_hbm.at[:, pl.ds(pl.multiple_of(q0 + hf * T2, T2), T2)], osem).start()

    for n in (1, 3, 0, 4, 6, 2, 5):
        mo[n] = _dot(_st_lhs(half_blk(wo_s), n), _st_rhs(oblk, n))
        fence()
        if n == 6:
            finish(0, mo[0] + mo[3] - mo[4] + mo[6], mo[1] + mo[3])
    finish(1, mo[2] + mo[4], mo[0] - mo[1] + mo[2] + mo[5])

    @pl.when(i == S // TQ - 1)
    def _():
        pltpu.make_async_copy(o_hbm, o_hbm, osem).wait()


@jax.jit
def pallas_gated_mix__mha_block__mixer_s_mlp__prompt_kernel(
    A_x: jax.Array,
    A_wqkv: jax.Array,
    A_wo: jax.Array,
    B_x: jax.Array,
    B_w1: jax.Array,
    B_w2: jax.Array,
    B_w3: jax.Array,
    B_w4: jax.Array,
    gate_w: jax.Array,
):
    del B_x
    xt = A_x.reshape(S, D).T
    vm = pltpu.VMEM
    out = pl.pallas_call(
        _kernel,
        grid=(S // TQ,),
        in_specs=[pl.BlockSpec(memory_space=pl.ANY)] * 8,
        out_specs=pl.BlockSpec(memory_space=pl.ANY),
        out_shape=jax.ShapeDtypeStruct((D, S), bf16),
        scratch_shapes=[
            vm((D, S), bf16), vm((D, 3 * D), bf16), vm((D, D), bf16), vm((D, D), bf16), vm((D, D), bf16),
            vm((D, F), bf16), vm((D, F), bf16), vm((D,), bf16), pltpu.SemaphoreType.DMA((13,)),
            vm((2, 3 * D, D2), bf16), vm((7, D2, D2), bf16), vm((2, D, D2), bf16), vm((2, D, D2), bf16),
            vm((26, D, G), bf16), vm((2, D, DP // 2), bf16), vm((D, 128), f32),
            vm((D, S), bf16), vm((4, S, 128), bf16), vm((H, HP, S), bf16),
            vm((D, S), f32), vm((D, S), f32), vm((H, HP, TQ), f32),
            vm((7, F2, T2), bf16), vm((2, 2, F2, T2), f32), vm((D, TQ), f32), vm((8, 128), f32),
            vm((S, W), f32), vm((S, W), f32),
            vm((S // TQ, 2, D, T2), bf16), pltpu.SemaphoreType.DMA(()),
        ],
        compiler_params=pltpu.CompilerParams(dimension_semantics=("arbitrary",),
                                             vmem_limit_bytes=100 * 1024 * 1024,
                                             disable_semaphore_checks=True, disable_bounds_checks=True),
        name="gm",
    )(xt, A_wqkv, A_wo, B_w1, B_w2, B_w3, B_w4.T, gate_w)
    return out.T.reshape(1, S, D)
```
